```python
import jax
import jax.numpy as jnp

def _softmax(x, axis=-1):
    return jax.nn.softmax(x, axis=axis)
def _gelu(x):
    return jax.nn.gelu(x, approximate=True)
def _silu(x):
    return jax.nn.silu(x)
def _sigmoid(x):
    return jax.nn.sigmoid(x)
def _layernorm(x, axis=-1, eps=1e-5):
    m = jnp.mean(x, axis=axis, keepdims=True)
    v = jnp.var(x, axis=axis, keepdims=True)
    return (x - m) / jnp.sqrt(v + eps)
def _scatter_add(tgt, idx, src, axis=0):
    return tgt.at[idx].add(src)
def _segment_sum(src, seg, n):
    return jax.ops.segment_sum(src, seg, n)
class _Rng:
    def __init__(self, key):
        self._k = key
    def _next(self):
        self._k, sub = jax.random.split(self._k)
        return sub
    def normal(self, shape):
        return jax.random.normal(self._next(), shape, dtype=jnp.bfloat16)
    def randint(self, lo, hi, shape):
        return jax.random.randint(self._next(), shape, lo, hi, dtype=jnp.int32)
    def uniform(self, shape, lo=0.0, hi=1.0):
        return jax.random.uniform(self._next(), shape, jnp.bfloat16, lo, hi)
    def permutation(self, n):
        return jax.random.permutation(self._next(), n)


kernel_name = 'interleave_layers__sliding_block__moe_arch_mod__prompt'

def setup_inputs():
    _rng = _Rng(jax.random.key(int.from_bytes(__import__("os").urandom(4), "little")))
    _w = (lambda a: (lambda t: t.astype(jnp.bfloat16) if jnp.issubdtype(t.dtype, jnp.floating) else t)(jnp.asarray(a)))
    def _A_setup():
        B, S, D = 1, 2048, 1024
        return {
            "x": _w((lambda *s: _rng.normal(s) * 0.05)(B, S, D)),
            "wqkv": _w((lambda *s: _rng.normal(s) * 0.05)(D, 3 * D)),
            "wo": _w((lambda *s: _rng.normal(s) * 0.05)(D, D)),
        }
    _A_in = _A_setup()

    def _B_setup():
        B, S, D, F, C = 1, 2048, 1024, 3584, 1
        return {
            "x": _w((lambda *s: _rng.normal(s) * 0.05)(B, S, D)),
            "w_r": _w((lambda *s: _rng.normal(s) * 0.05)(D)),
            "w_gate": _w((lambda *s: _rng.normal(s) * 0.05)(D, F)),
            "w_up": _w((lambda *s: _rng.normal(s) * 0.05)(D, F)),
            "w_down": _w((lambda *s: _rng.normal(s) * 0.05)(F, D)),
        }
    _B_in = _B_setup()

    return {
        "A_x": _A_in["x"],
        "A_wqkv": _A_in["wqkv"],
        "A_wo": _A_in["wo"],
        "B_x": _B_in["x"],
        "B_w_r": _B_in["w_r"],
        "B_w_gate": _B_in["w_gate"],
        "B_w_up": _B_in["w_up"],
        "B_w_down": _B_in["w_down"],
    }

def reference(A_x, A_wqkv, A_wo, B_x, B_w_r, B_w_gate, B_w_up, B_w_down):
    def _A_ref(x, wqkv, wo):
        B, S, D = x.shape
        H = 32; Dh = D // H; W = 256
        qkv = (lambda x, *d: x.transpose(*d))((x @ wqkv).reshape(B, S, 3, H, Dh), 2, 0, 3, 1, 4)
        q, k, v = qkv[0], qkv[1], qkv[2]
        scores = jnp.einsum("bhqd,bhkd->bhqk", q, k) * (Dh ** -0.5)
        idx = jnp.arange(S)
        mask = (idx[:, None] - idx[None, :] >= 0) & (idx[:, None] - idx[None, :] < W)
        scores = jnp.where(mask[None, None], scores, -1e9)
        p = _softmax(scores, axis=-1)
        o = jnp.einsum("bhqk,bhkd->bhqd", p, v)
        return (lambda x, *d: x.transpose(*d))(o, 0, 2, 1, 3).reshape(B, S, D) @ wo

    def _B_ref(x, w_r, w_gate, w_up, w_down):
        B, S, D = x.shape
        C = 1
        r = x @ w_r
        idx = jnp.argsort(-r, axis=-1)[:, :C]
        idx_e = jnp.repeat(idx.reshape(B, C, 1), D, axis=2)
        x_sel = jnp.take_along_axis(x, idx_e, axis=1)
        g = _silu(x_sel @ w_gate)
        u = x_sel @ w_up
        y = (g * u) @ w_down
        r_sel = _sigmoid(jnp.take_along_axis(r, idx, axis=1))
        y = y * r_sel.reshape(B, C, 1)
        b_off = (jnp.arange(B) * S).reshape(B, 1)
        flat_idx = (idx + b_off).reshape(B * C)
        zero = (x * 0.0).reshape(B * S, D)
        upd = _scatter_add(zero, flat_idx, y.reshape(B * C, D), axis=0)
        return x + upd.reshape(B, S, D)

    x = A_x
    x = x + _A_ref(_layernorm(x, axis=-1), A_wqkv, A_wo)
    x = x + _B_ref(_layernorm(x, axis=-1), B_w_r, B_w_gate, B_w_up, B_w_down)
    x = x + _A_ref(_layernorm(x, axis=-1), A_wqkv, A_wo)
    x = x + _B_ref(_layernorm(x, axis=-1), B_w_r, B_w_gate, B_w_up, B_w_down)
    return x
```

```python
import math

import jax
import jax.numpy as jnp
from jax import lax
import jax.experimental.pallas as pl
import jax.experimental.pallas.tpu as pltpu

S, D, F = 2048, 1024, 3584
DH = 32
HPG = 4
G = D // 128
R = 512
NQ = R // 128
NB = S // R
PR = R // G
NP = S // PR
NSTEP = NB * G
LAYERS = 2
EPS = 1e-5
CH = 16
NC = 128 // CH
QSCALE = DH ** -0.5 * math.log2(math.e)

bf16 = jnp.bfloat16
f32 = jnp.float32
u32 = jnp.uint32
i32 = jnp.int32


def _ln(x):
    m = jnp.mean(x, axis=-1, keepdims=True)
    xc = x - m
    v = jnp.mean(xc * xc, axis=-1, keepdims=True)
    return xc * lax.rsqrt(v + EPS)


def _dot(a, b):
    return jnp.dot(a, b, preferred_element_type=f32)


def _kernel(x_hbm, wqkv_hbm, wo_hbm, wr_ref, wg_hbm, wu_hbm, wd_hbm, out_hbm,
            x_s, h_s, acc_s, q_s, k_s, vt_s, o_s, wqkv_s, wo_s, wg_s, wu_s, wd_s,
            best_s, bidx_s, zero_s, sem_x, sem_w, sem_o):

    def x_in(b):
        rows = pl.ds(b * R, R)
        return pltpu.make_async_copy(x_hbm.at[rows], x_s.at[rows], sem_x.at[b])

    def wqkv_in(g):
        return [pltpu.make_async_copy(
            wqkv_hbm.at[:, pl.ds(t * D + g * 128, 128)], wqkv_s.at[g, t], sem_w.at[g])
            for t in range(3)]

    def wqkv_wait(g):
        pltpu.make_async_copy(wqkv_s.at[g], wqkv_s.at[g], sem_w.at[g]).wait()

    wo_in = pltpu.make_async_copy(wo_hbm, wo_s, sem_w.at[G])
    ffn_in = [pltpu.make_async_copy(a, b, sem_w.at[G + 1 + i]) for i, (a, b) in
              enumerate(((wg_hbm, wg_s), (wu_hbm, wu_s), (wd_hbm, wd_s)))]

    def x_out(b):
        rows = pl.ds(b * R, R)
        return pltpu.make_async_copy(x_s.at[rows], out_hbm.at[rows], sem_o.at[b])

    x_in(0).start()
    for c in wqkv_in(0):
        c.start()
    x_in(1).start()
    for c in wqkv_in(1):
        c.start()
    wo_in.start()
    for g in range(2, G):
        for c in wqkv_in(g):
            c.start()
    for b in range(2, NB):
        x_in(b).start()
    for c in ffn_in:
        c.start()
    zero_s[...] = jnp.zeros_like(zero_s)

    def rows_of(p, n):
        return pl.ds(p * n if isinstance(p, int) else pl.multiple_of(p * n, n), n)

    def ln_load(p):
        return x_s[rows_of(p, PR), :].astype(f32)

    def ln_store(x, p):
        h_s[rows_of(p, PR), :] = _ln(x).astype(bf16)
        acc_s[rows_of(p, PR), :] = x

    def epi_load(p):
        return acc_s[rows_of(p, PR), :]

    def epi_store(x1, p, pdst, valid):
        h1 = _ln(x1)
        x_s[rows_of(pdst, PR), :] = (x1 + h1).astype(bf16)
        r = jnp.sum(h1.astype(bf16).astype(f32) * wr_ref[...].astype(f32), axis=-1, keepdims=True)
        r = jnp.broadcast_to(r, (PR, 128))
        best, bidx = best_s[...], bidx_s[...]
        row = lax.broadcasted_iota(i32, (8, 128), 0) + p * PR
        for t in range(PR // 8):
            rt = r[t * 8:(t + 1) * 8]
            if valid is not None:
                rt = jnp.where(valid, rt, -jnp.inf)
            up = rt > best
            best = jnp.where(up, rt, best)
            bidx = jnp.where(up, row + t * 8, bidx)
        best_s[...] = best
        bidx_s[...] = bidx

    def proj_half(n, t, half):
        i, g = n // G, n % G
        ks = pl.ds(half * (D // 2), D // 2)
        return _dot(h_s[rows_of(i, R), ks], wqkv_s[g, t, ks, :])

    def proj_store(n, t, y):
        i, g = n // G, n % G
        if t == 0:
            q_s[n % 2] = (y * QSCALE).astype(bf16)
        elif t == 1:
            k_s[g, rows_of(i, R), :] = y.astype(bf16)
        else:
            for j in range(NQ):
                vt_s[g, i * NQ + j] = y[j * 128:(j + 1) * 128].T.astype(bf16)

    def oproj_half(n, o, half):
        i, g = n // G, n % G
        cs = pl.ds(half * (D // 2), D // 2)
        y = _dot(o, wo_s[g, :, cs])
        acc_s[rows_of(i, R), cs] += y
        return y

    def tri(c):
        return (lax.broadcasted_iota(i32, (CH, 128), 0) + c * CH
                <= lax.broadcasted_iota(i32, (CH, 128), 1))

    def attn_load(n, j, tiles):
        i, g = n // G, n % G
        qb = i * NQ + j
        q = q_s[n % 2, j * 128:(j + 1) * 128, :]
        kt = {t: k_s[g, rows_of(qb - t, 128), :] for t in tiles}
        k = jnp.concatenate([kt[t][c * CH:(c + 1) * CH] for c in range(NC) for t in tiles], axis=0)
        vt = jnp.concatenate([vt_s[g, qb - t] for t in tiles], axis=1)
        return q, k, vt

    def qk(q, k, h):
        qu = pltpu.bitcast(q, u32)
        lane = lax.broadcasted_iota(i32, qu.shape, 1)
        w = pltpu.bitcast(jnp.where(lane // DH == h, qu, jnp.zeros_like(qu)), bf16)
        return lax.dot_general(k, w, (((1,), (1,)), ((), ())), preferred_element_type=f32)

    def softmax(s, tiles, pace, zv):
        nt = len(tiles)
        diag, full, m = [], [], None
        for c in range(NC):
            part = {t: s[(nt * c + a) * CH:(nt * c + a + 1) * CH] for a, t in enumerate(tiles)}
            d = jnp.where(tri(c), part[0], part[2] if 2 in part else -jnp.inf)
            diag.append(d)
            if 1 in part:
                full.append(part[1])
                d = jnp.maximum(d, part[1])
            d = jnp.max(d.reshape(CH // 8, 8, 128), axis=0)
            m = d if m is None else jnp.maximum(m, d)
        m = jnp.broadcast_to(jnp.max(m, axis=0, keepdims=True), (8, 128))
        mu = pltpu.bitcast(m, u32)
        l, p = None, {t: [] for t in tiles}
        chunks = diag + full
        for c, x in enumerate(chunks):
            if pace is not None and c % 4 == 0:
                r0 = (c * pace.shape[0] // len(chunks)) // 8 * 8
                m = pltpu.bitcast(mu | (pltpu.bitcast(pace[r0:r0 + 8, 0:128], u32) & zv), f32)
            e = jnp.exp2(x.reshape(CH // 8, 8, 128) - m)
            t = jnp.sum(e, axis=0)
            l = t if l is None else l + t
            e = e.reshape(CH, 128)
            if c >= NC:
                p[1].append(e)
            elif 2 in p:
                e0 = jnp.where(tri(c), e, 0.0)
                p[0].append(e0)
                p[2].append(e - e0)
            else:
                p[0].append(e)
        p = jnp.concatenate([e for t in tiles for e in p[t]], axis=0)
        return p, jnp.sum(l, axis=0, keepdims=True)

    def step(n, first_block=False, proj=True, oproj=True, ln=True, epi=True):
        zv = zero_s[...]
        tiles = [(2, 0, 1)] * NQ
        if first_block:
            tiles = [(0,), (0, 1)] + tiles[2:]
        if epi:
            valid = n >= G + 1
            pe = jnp.maximum(n - (G + 1), 0)
            x1 = epi_load(pe)
        if ln:
            xl = ln_load(jnp.minimum(n + G + 1, NP - 1))
        loads = [attn_load(n, j, tiles[j]) for j in range(NQ)]

        fill = []
        if oproj:
            o_prev = o_s[(n - 1) % 2]
            fill += [lambda half=half: oproj_half(n - 1, o_prev, half) for half in range(2)]
        if proj:
            part = {}

            def run(t, half):
                y = proj_half(n + 1, t, half)
                if half:
                    proj_store(n + 1, t, part[t] + y)
                else:
                    part[t] = y
                return y
            fill += [lambda t=t, half=half: run(t, half) for t in (2, 1, 0) for half in range(2)]
        slots = [None] * (2 * NQ)
        order = list(range(0, 2 * NQ, 2)) + list(range(2 * NQ - 1, 0, -2))
        for a, f in zip(sorted(order[:len(fill)]), fill):
            slots[a] = f

        for j in range(NQ):
            q, k, vt = loads[j]
            ss = [qk(q, k, h) for h in range(HPG)]
            pace = slots[2 * j]() if slots[2 * j] else None
            sm = [softmax(s, tiles[j], pace, zv) for s in ss]
            ot = jnp.concatenate(
                [_dot(vt[h * DH:(h + 1) * DH], p.astype(bf16)) * (1.0 / l)
                 for h, (p, l) in enumerate(sm)], axis=0)
            o_s[n % 2, j * 128:(j + 1) * 128, :] = ot.T.astype(bf16)
            if slots[2 * j + 1]:
                slots[2 * j + 1]()

        if epi:
            epi_store(x1, pe, jnp.where(valid, pe, NP), valid)
        if ln:
            ln_store(xl, jnp.minimum(n + G + 1, NP))

    def layer(li, carry):
        first, last = li == 0, li == LAYERS - 1
        best_s[...] = jnp.full(best_s.shape, -jnp.inf, f32)
        bidx_s[...] = jnp.zeros_like(bidx_s)

        @pl.when(first)
        def _():
            x_in(0).wait()

        def ln_head(p, c):
            ln_store(ln_load(p), p)
            return c
        lax.fori_loop(0, G, ln_head, 0, unroll=2)

        @pl.when(first)
        def _():
            wqkv_wait(0)
            x_in(1).wait()

        xl = ln_load(G)
        for t in range(3):
            proj_store(0, t, proj_half(0, t, 0) + proj_half(0, t, 1))
        ln_store(xl, G)

        @pl.when(first)
        def _():
            wqkv_wait(1)

        step(0, first_block=True, oproj=False, epi=False)

        def head_body(n, c):
            @pl.when(first & (n == 1))
            def _():
                wo_in.wait()

            @pl.when(first & (n < G - 1))
            def _():
                wqkv_wait(n + 1)

            @pl.when(first & (n == G - 1))
            def _():
                for b in range(2, NB):
                    x_in(b).wait()

            step(n, first_block=True, epi=False)
            return c
        lax.fori_loop(1, G, head_body, 0)

        def body(n, c):
            for b in range(NB - 2):
                @pl.when(last & (n == G * (b + 2) + 1))
                def _():
                    x_out(b).start()

            step(n)
            return c
        lax.fori_loop(G, NSTEP - 1, body, 0)

        step(NSTEP - 1, proj=False, ln=False)
        x1 = epi_load(NP - G - 1)
        o_prev = o_s[(NSTEP - 1) % 2]
        for half in range(2):
            oproj_half(NSTEP - 1, o_prev, half)
        epi_store(x1, NP - G - 1, NP - G - 1, None)

        def epi_tail(p, c):
            epi_store(epi_load(p), p, p, None)
            return c
        lax.fori_loop(NP - G, NP, epi_tail, 0, unroll=2)

        @pl.when(last)
        def _():
            for b in range(NB - 2, NB):
                x_out(b).start()

        @pl.when(first)
        def _():
            for c in ffn_in:
                c.wait()

        best = best_s[...]
        top = jnp.max(best, axis=0, keepdims=True)
        idx = jnp.clip(jnp.min(jnp.where(best == top, bidx_s[...], S)), 0, S - 1)
        slab = rows_of(idx // 16, 16)
        sel = lax.broadcasted_iota(i32, (16, D), 0) == idx % 16
        hs = _ln(acc_s[slab, :]).astype(bf16)
        gate = _dot(hs, wg_s[...])
        up = _dot(hs, wu_s[...])
        y = _dot((gate * jax.nn.sigmoid(gate) * up).astype(bf16), wd_s[...])
        y = y * jax.nn.sigmoid(top[:, 0:1])

        @pl.when(last)
        def _():
            for b in range(NB):
                x_out(b).wait()

        xs = x_s[slab, :].astype(f32)
        x_s[slab, :] = jnp.where(sel, xs + y, xs).astype(bf16)

        @pl.when(last)
        def _():
            c = pltpu.make_async_copy(x_s.at[slab], out_hbm.at[slab], sem_o.at[0])
            c.start()
            c.wait()

        return carry

    lax.fori_loop(0, LAYERS, layer, 0)


@jax.jit
def pallas_interleave_layers__sliding_block__moe_arch_mod__prompt_kernel(
    A_x: jax.Array,
    A_wqkv: jax.Array,
    A_wo: jax.Array,
    B_x: jax.Array,
    B_w_r: jax.Array,
    B_w_gate: jax.Array,
    B_w_up: jax.Array,
    B_w_down: jax.Array,
):
    del B_x
    hbm = pl.BlockSpec(memory_space=pl.ANY)
    out = pl.pallas_call(
        _kernel,
        in_specs=[hbm, hbm, hbm, pl.BlockSpec(memory_space=pltpu.VMEM), hbm, hbm, hbm],
        out_specs=hbm,
        out_shape=jax.ShapeDtypeStruct((S, D), bf16),
        scratch_shapes=[
            pltpu.VMEM((S + PR, D), bf16),
            pltpu.VMEM((S + PR, D), bf16),
            pltpu.VMEM((S + PR, D), f32),
            pltpu.VMEM((2, R, 128), bf16),
            pltpu.VMEM((G, S, 128), bf16),
            pltpu.VMEM((G, S // 128, 128, 128), bf16),
            pltpu.VMEM((2, R, 128), bf16),
            pltpu.VMEM((G, 3, D, 128), bf16),
            pltpu.VMEM((G, 128, D), bf16),
            pltpu.VMEM((D, F), bf16),
            pltpu.VMEM((D, F), bf16),
            pltpu.VMEM((F, D), bf16),
            pltpu.VMEM((8, 128), f32),
            pltpu.VMEM((8, 128), i32),
            pltpu.VMEM((8, 128), u32),
            pltpu.SemaphoreType.DMA((NB,)),
            pltpu.SemaphoreType.DMA((G + 4,)),
            pltpu.SemaphoreType.DMA((NB,)),
        ],
        compiler_params=pltpu.CompilerParams(vmem_limit_bytes=100 * 1024 * 1024),
    )(A_x.reshape(S, D), A_wqkv, A_wo.reshape(G, 128, D), B_w_r.reshape(1, D),
      B_w_gate, B_w_up, B_w_down)
    return out.reshape(1, S, D)
```

```python
import math

import jax
import jax.numpy as jnp
from jax import lax
import jax.experimental.pallas as pl
import jax.experimental.pallas.tpu as pltpu

S, D, F = 2048, 1024, 3584
DH = 32
HPG = 4
G = D // 128
R = 512
NQ = R // 128
NB = S // R
PR = R // G
NP = S // PR
NSTEP = NB * G
LAYERS = 2
EPS = 1e-5
WIN = 256
NW = WIN // DH
PACE, PFRAC = 1, 0.7
UNROLL = 1
PLAN = {
    (True, True): "o0 s0 V0 e0 p0 s1 V1 e1 o1 p1 s2 K0 e2 K1 p2 s3 Q0 e3 p3 Q1",
    (True, False): "V0 s0 V1 e0 p0 s1 K0 e1 p1 s2 K1 e2 p2 s3 Q0 e3 p3 Q1",
    (False, True): "s0 s1 e0 p0 s2 e1 p1 s3 e2 p2 o0 e3 p3 o1",
}
QSCALE = DH ** -0.5 * math.log2(math.e)

bf16 = jnp.bfloat16
f32 = jnp.float32
u32 = jnp.uint32
i32 = jnp.int32


def _ln(x):
    m = jnp.mean(x, axis=-1, keepdims=True)
    xc = x - m
    v = jnp.mean(xc * xc, axis=-1, keepdims=True)
    return xc * lax.rsqrt(v + EPS)


def _dot(a, b):
    return jnp.dot(a, b, preferred_element_type=f32)


def _kernel(x_hbm, wqkv_hbm, wo_hbm, wr_ref, wg_hbm, wu_hbm, wd_hbm, out_hbm,
            x_s, h_s, acc_s, q_s, k_s, vt_s, o_s, wqkv_s, wo_s, wg_s, wu_s, wd_s,
            best_s, bidx_s, zero_s, sem_x, sem_w, sem_o):

    def x_in(b):
        rows = pl.ds(b * R, R)
        return pltpu.make_async_copy(x_hbm.at[rows], x_s.at[rows], sem_x.at[b])

    def wqkv_in(g):
        return [pltpu.make_async_copy(
            wqkv_hbm.at[:, pl.ds(t * D + g * 128, 128)], wqkv_s.at[g, t], sem_w.at[g])
            for t in range(3)]

    def wqkv_wait(g):
        pltpu.make_async_copy(wqkv_s.at[g], wqkv_s.at[g], sem_w.at[g]).wait()

    wo_in = pltpu.make_async_copy(wo_hbm, wo_s, sem_w.at[G])
    ffn_in = [pltpu.make_async_copy(a, b, sem_w.at[G + 1 + i]) for i, (a, b) in
              enumerate(((wg_hbm, wg_s), (wu_hbm, wu_s), (wd_hbm, wd_s.at[:, 0:D])))]

    def x_out(b):
        rows = pl.ds(b * R, R)
        return pltpu.make_async_copy(x_s.at[rows], out_hbm.at[rows], sem_o.at[b])

    x_in(0).start()
    for c in wqkv_in(0):
        c.start()
    zero_s[...] = jnp.zeros_like(zero_s)

    def rows_of(p, n):
        return pl.ds(p * n if isinstance(p, int) else pl.multiple_of(p * n, n), n)

    def ln_load(p):
        return x_s[rows_of(p, PR), :].astype(f32)

    def ln_store(x, p):
        h_s[rows_of(p, PR), :] = _ln(x).astype(bf16)
        acc_s[rows_of(p, PR), :] = x

    def epi_load(p):
        return acc_s[rows_of(p, PR), :]

    def epi_store(x1, p, pdst, valid):
        h1 = _ln(x1)
        x_s[rows_of(pdst, PR), :] = (x1 + h1).astype(bf16)
        r = jnp.sum(h1.astype(bf16).astype(f32) * wr_ref[...].astype(f32), axis=-1, keepdims=True)
        r = jnp.broadcast_to(r, (PR, 128))
        best, bidx = best_s[...], bidx_s[...]
        row = lax.broadcasted_iota(i32, (8, 128), 0) + p * PR
        for t in range(PR // 8):
            rt = r[t * 8:(t + 1) * 8]
            if valid is not None:
                rt = jnp.where(valid, rt, -jnp.inf)
            up = rt > best
            best = jnp.where(up, rt, best)
            bidx = jnp.where(up, row + t * 8, bidx)
        best_s[...] = best
        bidx_s[...] = bidx

    def proj_half(n, t, half):
        i, g = n // G, n % G
        ks = pl.ds(half * (D // 2), D // 2)
        return _dot(h_s[rows_of(i, R), ks], wqkv_s[g, t, ks, :])

    def proj_store(n, t, y):
        i, g = n // G, n % G
        if t == 0:
            q_s[n % 2] = (y * QSCALE).astype(bf16)
        elif t == 1:
            k_s[g, rows_of(i, R), :] = y.astype(bf16)
        else:
            for j in range(NQ):
                vt_s[g, i * NQ + j] = y[j * 128:(j + 1) * 128].T.astype(bf16)

    def oproj_half(n, o, half):
        i, g = n // G, n % G
        cs = pl.ds(half * (D // 2), D // 2)
        y = _dot(o, wo_s[g, :, cs])
        acc_s[rows_of(i, R), cs] += y
        return y

    def shift_sel(bit, hi, lo):
        if hi is None and lo is None:
            return None
        ref = lo if hi is None else hi
        lane = lax.broadcasted_iota(i32, ref.shape, 1)
        zero = jnp.zeros_like(ref)
        return jnp.where(lane & (DH * bit) != 0, zero if hi is None else hi,
                         zero if lo is None else lo)

    def lane_rolls(x):
        x = pltpu.bitcast(x, u32)
        return [x] + [pltpu.roll(x, DH * s, 1) for s in range(1, HPG)]

    def attn_load(n, first_block):
        i, g = n // G, n % G
        back = 0 if first_block else WIN // 128
        qr = lane_rolls(q_s[n % 2])
        kr = lane_rolls(k_s[g, pl.ds(pl.multiple_of(i * R - back * 128, 128), R + back * 128), :])
        vt = {t: vt_s[g, i * NQ + t] for t in range(-back, NQ)}
        lo = -back * HPG
        kc = [{c + lo: x[c * 16:(c + 1) * 16] for c in range(x.shape[0] // 16)} for x in kr]
        u = [{c: shift_sel(1, kc[(s + 1) % HPG].get(c + 1), kc[s].get(c))
              for c in range(-NW, R // DH - 1)} for s in range(HPG)]
        ks = [{c: shift_sel(2, u[(2 - h) % HPG][c + 2], u[-h % HPG][c])
               for c in range(-NW, R // DH - 3)} for h in range(HPG)]
        return qr, ks, vt

    def qk(qr, ks, j, h, chunks):
        w = []
        for a in range(HPG):
            x = qr[(a - h) % HPG][j * 64 + a * 16:j * 64 + (a + 1) * 16]
            lane = lax.broadcasted_iota(i32, x.shape, 1)
            w.append(jnp.where(lane // DH == a, x, jnp.zeros_like(x)))
        w = pltpu.bitcast(jnp.concatenate(w, axis=0), bf16)
        k = pltpu.bitcast(jnp.concatenate([ks[h][j * HPG - NW + c] for c in chunks], axis=0), bf16)
        s = lax.dot_general(k, w, (((1,), (1,)), ((), ())), preferred_element_type=f32)
        return {c: s[a * DH:(a + 1) * DH] for a, c in enumerate(chunks)}

    def softmax(s, start, pace, zv):
        lane = lax.broadcasted_iota(i32, (DH, 128), 1)
        tri = lax.broadcasted_iota(i32, (DH, 128), 0) <= lane % DH
        wrap = 0 in s
        s[NW] = jnp.where(tri, s[NW], s.pop(0) if wrap else -jnp.inf)
        m = None
        for c in s:
            if c < start:
                s[c] = jnp.where(lane // DH >= start - c, s[c], -jnp.inf)
            d = jnp.max(s[c].reshape(DH // 8, 8, 128), axis=0)
            m = d if m is None else jnp.maximum(m, d)
        m = jnp.broadcast_to(jnp.max(m, axis=0, keepdims=True), (8, 128))
        mu = pltpu.bitcast(m, u32)
        l, e = None, {}
        for a, c in enumerate(s):
            if pace is not None and a % PACE == 0:
                r0 = int(a * pace.shape[0] * PFRAC) // len(s) // 8 * 8
                m = pltpu.bitcast(mu | (pltpu.bitcast(pace[r0:r0 + 8, 0:128], u32) & zv), f32)
            x = jnp.exp2(s[c].reshape(DH // 8, 8, 128) - m)
            t = jnp.sum(x, axis=0)
            l = t if l is None else l + t
            e[c] = x.reshape(DH, 128)
        if wrap:
            x = e[NW]
            e[NW] = jnp.where(tri, x, 0.0)
            e[0] = x - e[NW]
        t = {c: shift_sel(1, e.get(c - 1), e.get(c)) for c in range(NW + 2)}
        p = {c: shift_sel(2, t.get(c - 2), t.get(c)) for c in range(max(start, 0), NW + HPG)}
        p = {c // HPG - WIN // 128: jnp.concatenate([p[c + a] for a in range(HPG)], axis=0)
             for c in range(max(start, 0), NW + HPG, HPG)}
        return p, jnp.sum(l, axis=0, keepdims=True)

    def step(n, first_block=False, proj=True, oproj=True, ln=True, epi=True):
        zv = zero_s[...]
        if epi:
            valid = n >= G + 1
            pe = jnp.maximum(n - (G + 1), 0)
            x1 = epi_load(pe)
        if ln:
            xl = ln_load(jnp.minimum(n + G + 1, NP - 1))
        qr, ks, vt = attn_load(n, first_block)
        if oproj:
            o_prev = o_s[(n - 1) % 2]
        part, ss, sm = {}, {}, {}
        pace = None

        for op in PLAN[proj, oproj].split():
            kind, j = op[0], int(op[1])
            start = NW - j * HPG if first_block else 0
            if kind == "o":
                pace = oproj_half(n - 1, o_prev, j)
            elif kind in "QKV":
                t = "QKV".index(kind)
                pace = proj_half(n + 1, t, j)
                if j:
                    proj_store(n + 1, t, part[t] + pace)
                part[t] = pace
            elif kind == "s":
                chunks = ([0] if start <= 0 else []) + [NW]
                chunks += range(max(start - HPG + 1, 1), NW)
                ss[j] = [qk(qr, ks, j, h, chunks) for h in range(HPG)]
                pace = None
            elif kind == "e":
                sm[j] = [softmax(s, start, pace, zv) for s in ss[j]]
            else:
                ot = [None] * HPG
                for t in sm[j][0][0]:
                    for h, (p, _) in enumerate(sm[j]):
                        y = _dot(vt[j + t][h * DH:(h + 1) * DH], p[t].astype(bf16))
                        ot[h] = y if ot[h] is None else ot[h] + y
                ot = jnp.concatenate([y * (1.0 / l) for y, (_, l) in zip(ot, sm[j])], axis=0)
                o_s[n % 2, j * 128:(j + 1) * 128, :] = ot.T.astype(bf16)

        if epi:
            epi_store(x1, pe, jnp.where(valid, pe, NP), valid)
        if ln:
            ln_store(xl, jnp.minimum(n + G + 1, NP))

    def layer(li, carry):
        first, last = li == 0, li == LAYERS - 1
        best_s[...] = jnp.full(best_s.shape, -jnp.inf, f32)
        bidx_s[...] = jnp.zeros_like(bidx_s)

        @pl.when(first)
        def _():
            x_in(0).wait()
            x_in(1).start()

        def ln_head(p, c):
            ln_store(ln_load(p), p)
            return c
        lax.fori_loop(0, G, ln_head, 0, unroll=2)

        @pl.when(first)
        def _():
            wqkv_wait(0)
            x_in(1).wait()
            for c in wqkv_in(1):
                c.start()

        xl = ln_load(G)
        for t in range(3):
            proj_store(0, t, proj_half(0, t, 0) + proj_half(0, t, 1))
        ln_store(xl, G)

        @pl.when(first)
        def _():
            wqkv_wait(1)
            wo_in.start()
            for c in wqkv_in(2):
                c.start()

        step(0, first_block=True, oproj=False, epi=False)

        def head_body(n, c):
            @pl.when(first & (n == 1))
            def _():
                wo_in.wait()
                for g in range(3, G):
                    for c in wqkv_in(g):
                        c.start()
                    if g == 3:
                        wqkv_wait(2)
                for b in range(2, NB):
                    x_in(b).start()

            @pl.when(first & (n > 1) & (n < G - 1))
            def _():
                wqkv_wait(n + 1)

            @pl.when(first & (n == G - 1))
            def _():
                for b in range(2, NB):
                    x_in(b).wait()
                for c in ffn_in:
                    c.start()

            step(n, first_block=True, epi=False)
            return c
        lax.fori_loop(1, G, head_body, 0)

        def body(n, c):
            for b in range(NB - 2):
                @pl.when(last & (n == G * (b + 2) + 1))
                def _():
                    x_out(b).start()

            step(n)
            return c
        lax.fori_loop(G, NSTEP - 1, body, 0, unroll=UNROLL)

        step(NSTEP - 1, proj=False, ln=False)
        x1 = epi_load(NP - G - 1)
        o_prev = o_s[(NSTEP - 1) % 2]
        for half in range(2):
            oproj_half(NSTEP - 1, o_prev, half)
        epi_store(x1, NP - G - 1, NP - G - 1, None)

        def epi_tail(p, c):
            epi_store(epi_load(p), p, p, None)
            return c
        lax.fori_loop(NP - G, NP, epi_tail, 0, unroll=2)

        @pl.when(last)
        def _():
            for b in range(NB - 2, NB):
                x_out(b).start()

        @pl.when(first)
        def _():
            for c in ffn_in:
                c.wait()

        best = best_s[...]
        top = jnp.max(best, axis=0, keepdims=True)
        idx = jnp.clip(jnp.min(jnp.where(best == top, bidx_s[...], S)), 0, S - 1)
        slab = rows_of(idx // 16, 16)
        sel = lax.broadcasted_iota(i32, (16, D), 0) == idx % 16
        hs = _ln(acc_s[slab, :]).astype(bf16)
        gate = _dot(hs, wg_s[...])
        up = _dot(hs, wu_s[...])
        y = _dot((gate * jax.nn.sigmoid(gate) * up).astype(bf16), wd_s[:, 0:D])
        y = y * jax.nn.sigmoid(top[:, 0:1])

        @pl.when(last)
        def _():
            for b in range(NB):
                x_out(b).wait()

        xs = x_s[slab, :].astype(f32)
        x_s[slab, :] = jnp.where(sel, xs + y, xs).astype(bf16)

        @pl.when(last)
        def _():
            c = pltpu.make_async_copy(x_s.at[slab], out_hbm.at[slab], sem_o.at[0])
            c.start()
            c.wait()

        return carry

    lax.fori_loop(0, LAYERS, layer, 0)


@jax.jit
def pallas_interleave_layers__sliding_block__moe_arch_mod__prompt_kernel(
    A_x: jax.Array,
    A_wqkv: jax.Array,
    A_wo: jax.Array,
    B_x: jax.Array,
    B_w_r: jax.Array,
    B_w_gate: jax.Array,
    B_w_up: jax.Array,
    B_w_down: jax.Array,
):
    del B_x
    hbm = pl.BlockSpec(memory_space=pl.ANY)
    out = pl.pallas_call(
        _kernel,
        in_specs=[hbm, hbm, hbm, pl.BlockSpec(memory_space=pltpu.VMEM), hbm, hbm, hbm],
        out_specs=hbm,
        out_shape=jax.ShapeDtypeStruct((S, D), bf16),
        scratch_shapes=[
            pltpu.VMEM((S + PR, D), bf16),
            pltpu.VMEM((S + PR, D), bf16),
            pltpu.VMEM((S + PR, D), f32),
            pltpu.VMEM((2, R, 128), bf16),
            pltpu.VMEM((G, S, 128), bf16),
            pltpu.VMEM((G, S // 128, 128, 128), bf16),
            pltpu.VMEM((2, R, 128), bf16),
            pltpu.VMEM((G, 3, D, 128), bf16),
            pltpu.VMEM((G, 128, D), bf16),
            pltpu.VMEM((D, F), bf16),
            pltpu.VMEM((D, F), bf16),
            pltpu.VMEM((F, D + 128), bf16),
            pltpu.VMEM((8, 128), f32),
            pltpu.VMEM((8, 128), i32),
            pltpu.VMEM((8, 128), u32),
            pltpu.SemaphoreType.DMA((NB,)),
            pltpu.SemaphoreType.DMA((G + 4,)),
            pltpu.SemaphoreType.DMA((NB,)),
        ],
        compiler_params=pltpu.CompilerParams(vmem_limit_bytes=100 * 1024 * 1024),
    )(A_x.reshape(S, D), A_wqkv, A_wo.reshape(G, 128, D), B_w_r.reshape(1, D),
      B_w_gate, B_w_up, B_w_down)
    return out.reshape(1, S, D)
```

```python
import math

import jax
import jax.numpy as jnp
from jax import lax
import jax.experimental.pallas as pl
import jax.experimental.pallas.tpu as pltpu

S, D, F = 2048, 1024, 3584
DH = 32
HPG = 4
G = D // 128
R = 512
NQ = R // 128
NB = S // R
PR = R // G
NP = S // PR
NSTEP = NB * G
LAYERS = 2
EPS = 1e-5
WIN = 256
NW = WIN // DH
PACE, PFRAC = 4, 0.7
LG = 3
HEAD_U, BODY_U = 2, 1
HS = 1
TB = 2
GATE, SGATE = 448, 1
PLAN_HEAD = "V0 s1 Q0 e1 p1 s2 V1 e2 p2 s0 Q1 e0 p0 N0 s3 K0 e3 p3 K1"
PLAN_BODY = "N0 o0 s0 V0 e0 p0 s1 V1 e1 p1 s2 K0 e2 o1 Q0 p2 s3 K1 e3 p3 Q1"
PLAN_LAST = ("o0 s0 o1 e0 p0 s1 O0 e1 p1 O1 s2 O2 e2 p2 O3 s3 O4 e3 p3 "
             "L0 O5 L1 O6 L2 O7 O8 L3 O9 L4 O10 L5 O11 O12 L6 O13 L7 O14 L8 O15")
LEAD = G + 1
QSCALE = DH ** -0.5 * math.log2(math.e)

bf16 = jnp.bfloat16
f32 = jnp.float32
u32 = jnp.uint32
i32 = jnp.int32


def _ln(x):
    m = jnp.mean(x, axis=-1, keepdims=True)
    xc = x - m
    v = jnp.mean(xc * xc, axis=-1, keepdims=True)
    return xc * lax.rsqrt(v + EPS)


def _dot(a, b):
    return jnp.dot(a, b, preferred_element_type=f32)


def _kernel(x_hbm, wqkv_hbm, wo_hbm, wr_ref, wg_hbm, wu_hbm, wd_hbm, out_hbm,
            x_s, h_s, h1_s, q_s, k_s, vt_s, o_s, wqkv_s, wo_s, wg_s, wu_s, wd_s,
            best_s, bidx_s, zero_s, sem_x, sem_w, sem_o):

    def x_in(b):
        rows = pl.ds(b * R, R)
        return pltpu.make_async_copy(x_hbm.at[rows], x_s.at[rows], sem_x.at[b])

    def wqkv_in(g):
        return [pltpu.make_async_copy(
            wqkv_hbm.at[:, pl.ds(t * D + g * 128, 128)], wqkv_s.at[g, t], sem_w.at[g])
            for t in range(3)]

    def wqkv_wait(g):
        pltpu.make_async_copy(wqkv_s.at[g], wqkv_s.at[g], sem_w.at[g]).wait()

    wo_in = pltpu.make_async_copy(wo_hbm, wo_s.at[:, 0:D], sem_w.at[G])
    ffn_in = [pltpu.make_async_copy(a, b, sem_w.at[G + 1 + i]) for i, (a, b) in
              enumerate(((wg_hbm, wg_s), (wu_hbm, wu_s), (wd_hbm, wd_s.at[:, 0:D])))]

    def x_out(b):
        rows = pl.ds(b * R, R)
        return pltpu.make_async_copy(x_s.at[rows], out_hbm.at[rows], sem_o.at[b])

    x_in(0).start()
    for c in wqkv_in(0):
        c.start()
    zero_s[...] = jnp.zeros_like(zero_s)

    def rows_of(p, n):
        return pl.ds(p * n if isinstance(p, int) else pl.multiple_of(p * n, n), n)

    def ln_load(p):
        return x_s[rows_of(p, PR), :].astype(f32)

    def ln_store(x, p):
        h_s[rows_of(p, PR), :] = _ln(x).astype(bf16)

    def epilogue(y, p):
        x1 = ln_load(p) + y
        h1 = _ln(x1)
        x_s[rows_of(p, PR), :] = (x1 + h1).astype(bf16)
        h1_s[rows_of(p, PR), :] = h1.astype(bf16)
        r = jnp.sum(h1 * wr_ref[...].astype(f32), axis=-1, keepdims=True)
        r = jnp.broadcast_to(r, (PR, 128))
        best, bidx = best_s[...], bidx_s[...]
        row = lax.broadcasted_iota(i32, (8, 128), 0) + p * PR
        for t in range(PR // 8):
            rt = r[t * 8:(t + 1) * 8]
            up = rt > best
            best = jnp.where(up, rt, best)
            bidx = jnp.where(up, row + t * 8, bidx)
        best_s[...] = best
        bidx_s[...] = bidx
        return bidx

    def proj_half(n, t, half, tok=None):
        i, g = n // G, n % G
        ks = pl.ds(half * (D // 2), D // 2)
        h = h_s[rows_of(i, R), ks]
        if tok is not None:
            x = pltpu.bitcast(h[GATE:GATE + 16], u32) | jnp.concatenate([tok] * (D // 256), axis=1)
            h = jnp.concatenate([h[:GATE], pltpu.bitcast(x, bf16), h[GATE + 16:]], axis=0)
        return _dot(h, wqkv_s[g, t, ks, :])

    def proj_store(n, t, y):
        i, g = n // G, n % G
        done = []
        if t == 0:
            q_s[n % 2] = (y * QSCALE).astype(bf16)
        elif t == 1:
            k_s[g, rows_of(i, R), :] = y.astype(bf16)
        else:
            for j in range(NQ):
                yt = y[j * 128:(j + 1) * 128]
                yt = yt.astype(bf16).T if TB > 1 else yt.T.astype(bf16)
                vt_s[g, i * NQ + j] = yt
                done.append(yt)
        return done

    def o_load(p, rows=PR):
        return jnp.concatenate([o_s[g, rows_of(p, rows), :] for g in range(G)], axis=1)

    def oproj_part(o, part):
        cols = D * PR // (2 * o.shape[0])
        return _dot(o, wo_s[:, pl.ds(part * cols, cols)])

    def shift_sel(bit, hi, lo):
        if hi is None and lo is None:
            return None
        ref = lo if hi is None else hi
        lane = lax.broadcasted_iota(i32, ref.shape, 1)
        zero = jnp.zeros_like(ref)
        return jnp.where(lane & (DH * bit) != 0, zero if hi is None else hi,
                         zero if lo is None else lo)

    def lane_rolls(x):
        x = pltpu.bitcast(x, u32)
        return [x] + [pltpu.roll(x, DH * s, 1) for s in range(1, HPG)]

    def attn_load(n, first_block):
        i, g = n // G, n % G
        back = 0 if first_block else WIN // 128
        qr = lane_rolls(q_s[n % 2])
        kr = lane_rolls(k_s[g, pl.ds(pl.multiple_of(i * R - back * 128, 128), R + back * 128), :])
        vt = {t: vt_s[g, i * NQ + t] for t in range(-back, NQ)}
        lo = -back * HPG
        kc = [{c + lo: x[c * 16:(c + 1) * 16] for c in range(x.shape[0] // 16)} for x in kr]
        u = [{c: shift_sel(1, kc[(s + 1) % HPG].get(c + 1), kc[s].get(c))
              for c in range(-NW, R // DH - 1)} for s in range(HPG)]
        ks = [{c: shift_sel(2, u[(2 - h) % HPG][c + 2], u[-h % HPG][c])
               for c in range(-NW, R // DH - 3)} for h in range(HPG)]
        return qr, ks, vt

    def qk(qr, ks, j, h, chunks, tok):
        w = []
        for a in range(HPG):
            x = qr[(a - h) % HPG][j * 64 + a * 16:j * 64 + (a + 1) * 16]
            lane = lax.broadcasted_iota(i32, x.shape, 1)
            w.append(jnp.where(lane // DH == a, x, jnp.zeros_like(x)))
        if tok is not None:
            w[0] = w[0] | jnp.concatenate([tok] * 2, axis=0)
        w = pltpu.bitcast(jnp.concatenate(w, axis=0), bf16)
        k = pltpu.bitcast(jnp.concatenate([ks[h][j * HPG - NW + c] for c in chunks], axis=0), bf16)
        s = lax.dot_general(k, w, (((1,), (1,)), ((), ())), preferred_element_type=f32)
        return {c: s[a * DH:(a + 1) * DH] for a, c in enumerate(chunks)}

    def softmax(ss, start, pace, zv):
        lane = lax.broadcasted_iota(i32, (DH, 128), 1)
        tri = lax.broadcasted_iota(i32, (DH, 128), 0) <= lane % DH
        wrap = 0 in ss[0]
        ms = []
        for s in ss:
            s[NW] = jnp.where(tri, s[NW], s.pop(0) if wrap else -jnp.inf)
            m = None
            for c in s:
                if c < start:
                    s[c] = jnp.where(lane // DH >= start - c, s[c], -jnp.inf)
                d = jnp.max(s[c].reshape(DH // 8, 8, 128), axis=0)
                m = d if m is None else jnp.maximum(m, d)
            ms.append(jnp.broadcast_to(jnp.max(m, axis=0, keepdims=True), (8, 128)))
        ls, es, mp = [None] * len(ss), [{} for _ in ss], list(ms)
        for a, c in enumerate(ss[0]):
            for h, s in enumerate(ss):
                if pace is not None and a % PACE == 0:
                    pr = pace.shape[0]
                    r0 = int((a + HS * PACE * h / len(ss)) * pace.size // 128 * PFRAC) // len(s) // 8 * 8
                    src = pace[r0 % pr:r0 % pr + 8, r0 // pr * 128:(r0 // pr + 1) * 128]
                    mp[h] = pltpu.bitcast(
                        pltpu.bitcast(ms[h], u32) | (pltpu.bitcast(src, u32) & zv), f32)
                x = jnp.exp2(s[c].reshape(DH // 8, 8, 128) - mp[h])
                t = jnp.sum(x, axis=0)
                ls[h] = t if ls[h] is None else ls[h] + t
                es[h][c] = x.reshape(DH, 128)
        out = []
        for e, l in zip(es, ls):
            if wrap:
                x = e[NW]
                e[NW] = jnp.where(tri, x, 0.0)
                e[0] = x - e[NW]
            t = {c: shift_sel(1, e.get(c - 1), e.get(c)) for c in range(NW + 2)}
            p = {c: shift_sel(2, t.get(c - 2), t.get(c)) for c in range(max(start, 0), NW + HPG)}
            p = {c // HPG - WIN // 128: jnp.concatenate([p[c + a] for a in range(HPG)], axis=0)
                 for c in range(max(start, 0), NW + HPG, HPG)}
            out.append((p, jnp.sum(l, axis=0, keepdims=True)))
        return out

    def steps(n0, plans, first_block=False):
        pn = [jnp.minimum(n0 + LEAD + a, NP - 1) for a in range(len(plans))]
        xl = [ln_load(p) if "N" in plan else None for p, plan in zip(pn, plans)]
        oi = [o_load(n0 - G + a) if "o" in plan else None for a, plan in enumerate(plans)]
        due = []
        for a, plan in enumerate(plans):
            step(n0 + a, plan, first_block, xl[a], pn[a], oi[a], due)

    def step(n, plan, first_block, xl, pn, oi, due):
        zv = zero_s[...]
        qr, ks, vt = attn_load(n, first_block)
        part, ss, sm = {}, {}, {}
        pace, late = None, []

        def settle():
            if not due:
                return None
            tok = zv
            for x in due:
                tok = tok & pltpu.bitcast(x[-16:], u32)
            due.clear()
            return tok

        for op in plan.split():
            kind, j = op[0], int(op[1:])
            start = NW - j * HPG if first_block else 0
            if kind == "o":
                pace = oproj_part(oi, j)
                if j:
                    late.append(epilogue(jnp.concatenate([part["o"], pace], axis=1), n - G))
                part["o"] = pace
            elif kind == "O":
                tile = (NB - 1) * NQ + j // 4
                o = o_load(tile, 128)
                if late and j % 4 == LG:
                    tok = zv
                    for x in late:
                        tok = tok & pltpu.bitcast(x, u32)
                    late.clear()
                    o = pltpu.bitcast(o, u32)
                    o = pltpu.bitcast(jnp.concatenate(
                        [o[:-8], o[-8:] | jnp.concatenate([tok] * G, axis=1)], axis=0), bf16)
                part[j % 4] = pace = oproj_part(o, j % 4)
                if j % 4 == 3:
                    y = jnp.concatenate([part[a] for a in range(4)], axis=1)
                    for a in range(128 // PR):
                        late.append(epilogue(y[a * PR:(a + 1) * PR], tile * 128 // PR + a))
            elif kind == "N":
                ln_store(xl, pn)
            elif kind == "L":
                ln_store(ln_load(j), j)
            elif kind in "QKV":
                t = "QKV".index(kind)
                pace = proj_half(n + 1, t, j, settle())
                if j:
                    due.extend(proj_store(n + 1, t, part[t] + pace))
                part[t] = pace
            elif kind == "s":
                chunks = ([0] if start <= 0 else []) + [NW]
                chunks += range(max(start - HPG + 1, 1), NW)
                tok = None
                if SGATE and pace is not None:
                    tok = pltpu.bitcast(pace[0:8, 0:128], u32) & zv
                ss[j] = [qk(qr, ks, j, h, chunks, tok) for h in range(HPG)]
                pace = None
            elif kind == "e":
                sm[j] = softmax(ss[j], start, pace, zv)
            else:
                ot = [None] * HPG
                for t in sm[j][0][0]:
                    for h, (p, _) in enumerate(sm[j]):
                        y = _dot(vt[j + t][h * DH:(h + 1) * DH], p[t].astype(bf16))
                        ot[h] = y if ot[h] is None else ot[h] + y
                ot = jnp.concatenate([y * (1.0 / l) for y, (_, l) in zip(ot, sm[j])], axis=0)
                ot = ot.astype(bf16).T if TB else ot.T.astype(bf16)
                o_s[n % G, rows_of((n // G) * NQ + j, 128), :] = ot
                due.append(ot)


    x_in(0).wait()
    x_in(1).start()

    def ln_head(p, c):
        ln_store(ln_load(p), p)
        return c
    lax.fori_loop(0, G, ln_head, 0, unroll=2)
    x_in(1).wait()
    ln_head(G, 0)
    wqkv_wait(0)
    for g in range(1, 1 + HEAD_U):
        for c in wqkv_in(g):
            c.start()

    def layer(li, carry):
        first, last = li == 0, li == LAYERS - 1
        best_s[...] = jnp.full(best_s.shape, -jnp.inf, f32)
        bidx_s[...] = jnp.zeros_like(bidx_s)

        for t in (1, 0, 2):
            proj_store(0, t, proj_half(0, t, 0) + proj_half(0, t, 1))

        def head_body(a, c):
            n = a * HEAD_U
            for n0 in range(0, G, HEAD_U):
                @pl.when(first & (n == n0))
                def _():
                    for g in range(n0 + 1, min(n0 + 1 + HEAD_U, G)):
                        wqkv_wait(g)
                    for g in range(n0 + 1 + HEAD_U, min(n0 + 1 + 2 * HEAD_U, G)):
                        for c in wqkv_in(g):
                            c.start()
                    if n0 == 0:
                        x_in(2).start()
                    if n0 <= 2 * G - LEAD < n0 + HEAD_U:
                        x_in(2).wait()
                    if n0 == G - HEAD_U:
                        wo_in.start()
                        for b in range(3, NB):
                            x_in(b).start()

            steps(n, [PLAN_HEAD] * HEAD_U, first_block=True)
            return c
        lax.fori_loop(0, G // HEAD_U, head_body, 0)

        @pl.when(first)
        def _():
            wo_in.wait()
            for b in range(3, NB):
                x_in(b).wait()
            for c in ffn_in:
                c.start()

        def body(a, c):
            n = a * BODY_U
            for b in range(NB - 2):
                @pl.when(last & (n == G * (b + 2)))
                def _():
                    x_out(b).start()

            steps(n, [PLAN_BODY] * BODY_U)
            return c
        lax.fori_loop(G // BODY_U, NSTEP // BODY_U - 1, body, 0)

        steps(NSTEP - BODY_U, [PLAN_BODY.replace("N0 ", "")] * (BODY_U - 1) + [PLAN_LAST])

        @pl.when(last)
        def _():
            for b in range(NB - 2, NB):
                x_out(b).start()

        @pl.when(first)
        def _():
            for c in ffn_in:
                c.wait()

        best = best_s[...]
        top = jnp.max(best, axis=0, keepdims=True)
        idx = jnp.clip(jnp.min(jnp.where(best == top, bidx_s[...], S)), 0, S - 1)
        slab = rows_of(idx // 16, 16)
        sel = lax.broadcasted_iota(i32, (16, D), 0) == idx % 16
        hs = h1_s[slab, :]
        gate = _dot(hs, wg_s[...])
        up = _dot(hs, wu_s[...])
        y = _dot((gate * jax.nn.sigmoid(gate) * up).astype(bf16), wd_s[:, 0:D])
        y = y * jax.nn.sigmoid(top[:, 0:1])

        @pl.when(last)
        def _():
            for b in range(NB):
                x_out(b).wait()

        xs = x_s[slab, :].astype(f32)
        xs = jnp.where(sel, xs + y, xs).astype(bf16)
        x_s[slab, :] = xs

        @pl.when(last)
        def _():
            c = pltpu.make_async_copy(x_s.at[slab], out_hbm.at[slab], sem_o.at[0])
            c.start()
            c.wait()

        h_s[slab, :] = _ln(xs.astype(f32)).astype(bf16)
        return carry

    lax.fori_loop(0, LAYERS, layer, 0)


@jax.jit
def pallas_interleave_layers__sliding_block__moe_arch_mod__prompt_kernel(
    A_x: jax.Array,
    A_wqkv: jax.Array,
    A_wo: jax.Array,
    B_x: jax.Array,
    B_w_r: jax.Array,
    B_w_gate: jax.Array,
    B_w_up: jax.Array,
    B_w_down: jax.Array,
):
    del B_x
    hbm = pl.BlockSpec(memory_space=pl.ANY)
    out = pl.pallas_call(
        _kernel,
        in_specs=[hbm, hbm, hbm, pl.BlockSpec(memory_space=pltpu.VMEM), hbm, hbm, hbm],
        out_specs=hbm,
        out_shape=jax.ShapeDtypeStruct((S, D), bf16),
        scratch_shapes=[
            pltpu.VMEM((S, D), bf16),
            pltpu.VMEM((S, D), bf16),
            pltpu.VMEM((S, D), bf16),
            pltpu.VMEM((2, R, 128), bf16),
            pltpu.VMEM((G, S, 128), bf16),
            pltpu.VMEM((G, S // 128, 128, 128), bf16),
            pltpu.VMEM((G, S, 128), bf16),
            pltpu.VMEM((G, 3, D, 128), bf16),
            pltpu.VMEM((D, D + 128), bf16),
            pltpu.VMEM((D, F), bf16),
            pltpu.VMEM((D, F), bf16),
            pltpu.VMEM((F, D + 128), bf16),
            pltpu.VMEM((8, 128), f32),
            pltpu.VMEM((8, 128), i32),
            pltpu.VMEM((8, 128), u32),
            pltpu.SemaphoreType.DMA((NB,)),
            pltpu.SemaphoreType.DMA((G + 4,)),
            pltpu.SemaphoreType.DMA((NB,)),
        ],
        compiler_params=pltpu.CompilerParams(vmem_limit_bytes=100 * 1024 * 1024),
    )(A_x.reshape(S, D), A_wqkv, A_wo, B_w_r.reshape(1, D),
      B_w_gate, B_w_up, B_w_down)
    return out.reshape(1, S, D)
```

```python
import math

import jax
import jax.numpy as jnp
from jax import lax
import jax.experimental.pallas as pl
import jax.experimental.pallas.tpu as pltpu

S, D, F = 2048, 1024, 3584
DH = 32
HPG = 4
G = D // 128
R = 512
NQ = R // 128
NB = S // R
PR = R // G
NP = S // PR
NSTEP = NB * G
LAYERS = 2
EPS = 1e-5
WIN = 256
NW = WIN // DH
PACE, PFRAC = 4, 0.7
LG = 99
XB = 4
HEAD_U, BODY_U = 2, 1
HS = 1
TB = 2
GATE, SGATE = 448, 1
PLAN_HEAD = "V0 s1 Q0 e1 p1 s2 V1 e2 p2 s0 Q1 e0 p0 N0 s3 K0 e3 p3 K1"
PLAN_BODY = "N0 o0 s0 V0 e0 p0 s1 V1 e1 p1 s2 K0 e2 o1 Q0 p2 s3 K1 e3 p3 Q1"
PLAN_LAST = ("N0 o0 s0 o1 e0 p0 s1 o2 e1 o3 p1 s2 o4 e2 o5 p2 s3 o6 e3 o7 p3 "
             "o8 o9 o10 o11 o12 o13 o14 o15 o16 o17")
LEAD = G + 1
QSCALE = DH ** -0.5 * math.log2(math.e)

bf16 = jnp.bfloat16
f32 = jnp.float32
u32 = jnp.uint32
i32 = jnp.int32


def _ln(x):
    m = jnp.mean(x, axis=-1, keepdims=True)
    xc = x - m
    v = jnp.mean(xc * xc, axis=-1, keepdims=True)
    return xc * lax.rsqrt(v + EPS)


def _dot(a, b):
    return jnp.dot(a, b, preferred_element_type=f32)


def _kernel(x_hbm, wqkv_hbm, wo_hbm, wr_ref, wg_hbm, wu_hbm, wd_hbm, out_hbm,
            x_s, h_s, h1_s, q_s, k_s, vt_s, o_s, wqkv_s, wo_s, wg_s, wu_s, wd_s,
            best_s, bidx_s, zero_s, wr_s, sem_x, sem_w, sem_o):

    def x_in(b):
        lo, hi = (LEAD * PR if b == 1 else b * R), (LEAD * PR if b == 0 else (b + 1) * R)
        rows = pl.ds(lo, hi - lo)
        return pltpu.make_async_copy(x_hbm.at[rows], x_s.at[rows], sem_x.at[b])

    def wqkv_in(g):
        return [pltpu.make_async_copy(
            wqkv_hbm.at[:, pl.ds(t * D + g * 128, 128)], wqkv_s.at[g, t], sem_w.at[g])
            for t in range(3)]

    def wqkv_wait(g):
        pltpu.make_async_copy(wqkv_s.at[g], wqkv_s.at[g], sem_w.at[g]).wait()

    wo_in = pltpu.make_async_copy(wo_hbm, wo_s.at[:, 0:D], sem_w.at[G])
    ffn_in = [pltpu.make_async_copy(a, b, sem_w.at[G + 1 + i]) for i, (a, b) in
              enumerate(((wg_hbm, wg_s), (wu_hbm, wu_s), (wd_hbm, wd_s.at[:, 0:D])))]

    def x_out(b):
        rows = pl.ds(b * R, R)
        return pltpu.make_async_copy(x_s.at[rows], out_hbm.at[rows], sem_o.at[b])

    x_in(0).start()
    wr_s[...] = jnp.broadcast_to(wr_ref[...].astype(f32).reshape(1, D), (8, D))
    zero_s[...] = jnp.zeros_like(zero_s)

    def rows_of(p, n):
        return pl.ds(p * n if isinstance(p, int) else pl.multiple_of(p * n, n), n)

    def ln_load(p):
        return x_s[rows_of(p, PR), :].astype(f32)

    def ln_store(x, p):
        h_s[rows_of(p, PR), :] = _ln(x).astype(bf16)

    def epilogue(y, p):
        x1 = ln_load(p) + y
        xc = x1 - jnp.mean(x1, axis=-1, keepdims=True)
        rstd = lax.rsqrt(jnp.mean(xc * xc, axis=-1, keepdims=True) + EPS)
        r = jnp.sum(xc * wr_s[0:1, :], axis=-1, keepdims=True) * rstd
        h1 = xc * rstd
        xb = (x1 + h1).astype(bf16)
        x_s[rows_of(p, PR), :] = xb
        h1_s[rows_of(p, PR), :] = h1.astype(bf16)
        r = jnp.broadcast_to(r, (PR, 128))
        best, bidx = best_s[...], bidx_s[...]
        row = lax.broadcasted_iota(i32, (8, 128), 0) + p * PR
        for t in range(PR // 8):
            rt = r[t * 8:(t + 1) * 8]
            up = rt > best
            best = jnp.where(up, rt, best)
            bidx = jnp.where(up, row + t * 8, bidx)
        best_s[...] = best
        bidx_s[...] = bidx
        return [bidx] + [xb[:r] for r in range(16, PR + 1, 16)][:XB]

    def proj_half(n, t, half, tok=None):
        i, g = n // G, n % G
        ks = pl.ds(half * (D // 2), D // 2)
        h = h_s[rows_of(i, R), ks]
        if tok is not None:
            x = pltpu.bitcast(h[GATE:GATE + 16], u32) | jnp.concatenate([tok] * (D // 256), axis=1)
            h = jnp.concatenate([h[:GATE], pltpu.bitcast(x, bf16), h[GATE + 16:]], axis=0)
        return _dot(h, wqkv_s[g, t, ks, :])

    def proj_store(n, t, y):
        i, g = n // G, n % G
        done = []
        if t == 0:
            q_s[n % 2] = (y * QSCALE).astype(bf16)
        elif t == 1:
            k_s[g, rows_of(i, R), :] = y.astype(bf16)
        else:
            for j in range(NQ):
                yt = y[j * 128:(j + 1) * 128]
                yt = yt.astype(bf16).T if TB > 1 else yt.T.astype(bf16)
                vt_s[g, i * NQ + j] = yt
                done.append(yt)
        return done

    def o_load(p):
        return jnp.concatenate([o_s[g, rows_of(p, PR), :] for g in range(G)], axis=1)

    def oproj_half(o, half):
        return _dot(o, wo_s[:, pl.ds(half * (D // 2), D // 2)])

    def shift_sel(bit, hi, lo):
        if hi is None and lo is None:
            return None
        ref = lo if hi is None else hi
        lane = lax.broadcasted_iota(i32, ref.shape, 1)
        zero = jnp.zeros_like(ref)
        return jnp.where(lane & (DH * bit) != 0, zero if hi is None else hi,
                         zero if lo is None else lo)

    def lane_rolls(x):
        x = pltpu.bitcast(x, u32)
        return [x] + [pltpu.roll(x, DH * s, 1) for s in range(1, HPG)]

    def attn_load(n, first_block):
        i, g = n // G, n % G
        back = 0 if first_block else WIN // 128
        qr = lane_rolls(q_s[n % 2])
        kr = lane_rolls(k_s[g, pl.ds(pl.multiple_of(i * R - back * 128, 128), R + back * 128), :])
        vt = {t: vt_s[g, i * NQ + t] for t in range(-back, NQ)}
        lo = -back * HPG
        kc = [{c + lo: x[c * 16:(c + 1) * 16] for c in range(x.shape[0] // 16)} for x in kr]
        u = [{c: shift_sel(1, kc[(s + 1) % HPG].get(c + 1), kc[s].get(c))
              for c in range(-NW, R // DH - 1)} for s in range(HPG)]
        ks = [{c: shift_sel(2, u[(2 - h) % HPG][c + 2], u[-h % HPG][c])
               for c in range(-NW, R // DH - 3)} for h in range(HPG)]
        return qr, ks, vt

    def qk(qr, ks, j, h, chunks, tok):
        w = []
        for a in range(HPG):
            x = qr[(a - h) % HPG][j * 64 + a * 16:j * 64 + (a + 1) * 16]
            lane = lax.broadcasted_iota(i32, x.shape, 1)
            w.append(jnp.where(lane // DH == a, x, jnp.zeros_like(x)))
        if tok is not None:
            w[0] = w[0] | jnp.concatenate([tok] * 2, axis=0)
        w = pltpu.bitcast(jnp.concatenate(w, axis=0), bf16)
        k = pltpu.bitcast(jnp.concatenate([ks[h][j * HPG - NW + c] for c in chunks], axis=0), bf16)
        s = lax.dot_general(k, w, (((1,), (1,)), ((), ())), preferred_element_type=f32)
        return {c: s[a * DH:(a + 1) * DH] for a, c in enumerate(chunks)}

    def softmax(ss, start, pace, zv):
        lane = lax.broadcasted_iota(i32, (DH, 128), 1)
        tri = lax.broadcasted_iota(i32, (DH, 128), 0) <= lane % DH
        wrap = 0 in ss[0]
        ms = []
        for s in ss:
            s[NW] = jnp.where(tri, s[NW], s.pop(0) if wrap else -jnp.inf)
            m = None
            for c in s:
                if c < start:
                    s[c] = jnp.where(lane // DH >= start - c, s[c], -jnp.inf)
                d = jnp.max(s[c].reshape(DH // 8, 8, 128), axis=0)
                m = d if m is None else jnp.maximum(m, d)
            ms.append(jnp.broadcast_to(jnp.max(m, axis=0, keepdims=True), (8, 128)))
        ls, es, mp = [None] * len(ss), [{} for _ in ss], list(ms)
        for a, c in enumerate(ss[0]):
            for h, s in enumerate(ss):
                if pace is not None and a % PACE == 0:
                    pr = pace.shape[0]
                    r0 = int((a + HS * PACE * h / len(ss)) * pace.size // 128 * PFRAC) // len(s) // 8 * 8
                    src = pace[r0 % pr:r0 % pr + 8, r0 // pr * 128:(r0 // pr + 1) * 128]
                    mp[h] = pltpu.bitcast(
                        pltpu.bitcast(ms[h], u32) | (pltpu.bitcast(src, u32) & zv), f32)
                x = jnp.exp2(s[c].reshape(DH // 8, 8, 128) - mp[h])
                t = jnp.sum(x, axis=0)
                ls[h] = t if ls[h] is None else ls[h] + t
                es[h][c] = x.reshape(DH, 128)
        out = []
        for e, l in zip(es, ls):
            if wrap:
                x = e[NW]
                e[NW] = jnp.where(tri, x, 0.0)
                e[0] = x - e[NW]
            t = {c: shift_sel(1, e.get(c - 1), e.get(c)) for c in range(NW + 2)}
            p = {c: shift_sel(2, t.get(c - 2), t.get(c)) for c in range(max(start, 0), NW + HPG)}
            p = {c // HPG - WIN // 128: jnp.concatenate([p[c + a] for a in range(HPG)], axis=0)
                 for c in range(max(start, 0), NW + HPG, HPG)}
            out.append((p, jnp.sum(l, axis=0, keepdims=True)))
        return out

    def steps(n0, plans, first_block=False):
        pn = [(n0 + LEAD + a) % NP for a in range(len(plans))]
        xl = [ln_load(p) if "N" in plan else None for p, plan in zip(pn, plans)]
        oi = [o_load(n0 - G + a) if "o" in plan else None for a, plan in enumerate(plans)]
        due = []
        for a, plan in enumerate(plans):
            step(n0 + a, plan, first_block, xl[a], pn[a], oi[a], due)

    def step(n, plan, first_block, xl, pn, oi, due):
        zv = zero_s[...]
        qr, ks, vt = attn_load(n, first_block)
        part, ss, sm = {}, {}, {}
        pace = None

        def settle():
            now = [x for wait, x in due if wait == 0]
            due[:] = [(wait - 1, x) for wait, x in due if wait]
            tok = zv if now else None
            for x in now:
                tok = tok & pltpu.bitcast(x[-32 // x.dtype.itemsize:, -128:], u32)
            return tok

        for op in plan.split():
            kind, j = op[0], int(op[1:])
            start = NW - j * HPG if first_block else 0
            if kind == "o":
                piece = n - G + j // 2
                if j > 1 and j % 2 == 0:
                    oi = o_load(piece)
                pace = oproj_half(oi, j % 2)
                if j % 2:
                    done = epilogue(jnp.concatenate([part["o"], pace], axis=1), piece)
                    due.extend((LG, x) for x in done)
                part["o"] = pace
            elif kind == "N":
                ln_store(xl, pn)
            elif kind in "QKV":
                t = "QKV".index(kind)
                pace = proj_half(n + 1, t, j, settle())
                if j:
                    due.extend((0, x) for x in proj_store(n + 1, t, part[t] + pace))
                part[t] = pace
            elif kind == "s":
                chunks = ([0] if start <= 0 else []) + [NW]
                chunks += range(max(start - HPG + 1, 1), NW)
                tok = None
                if SGATE and pace is not None:
                    tok = pltpu.bitcast(pace[0:8, 0:128], u32) & zv
                ss[j] = [qk(qr, ks, j, h, chunks, tok) for h in range(HPG)]
                pace = None
            elif kind == "e":
                sm[j] = softmax(ss[j], start, pace, zv)
            else:
                ot = [None] * HPG
                for t in sm[j][0][0]:
                    for h, (p, _) in enumerate(sm[j]):
                        y = _dot(vt[j + t][h * DH:(h + 1) * DH], p[t].astype(bf16))
                        ot[h] = y if ot[h] is None else ot[h] + y
                ot = jnp.concatenate([y * (1.0 / l) for y, (_, l) in zip(ot, sm[j])], axis=0)
                ot = ot.astype(bf16).T if TB else ot.T.astype(bf16)
                o_s[n % G, rows_of((n // G) * NQ + j, 128), :] = ot
                due.append((0, ot))


    x_in(0).wait()
    for c in wqkv_in(0):
        c.start()

    def ln_head(p, c):
        ln_store(ln_load(p), p)
        return c
    lax.fori_loop(0, LEAD, ln_head, 0, unroll=3)
    wqkv_wait(0)
    x_in(1).start()
    for g in range(1, 1 + HEAD_U):
        for c in wqkv_in(g):
            c.start()

    def layer(li, carry):
        first, last = li == 0, li == LAYERS - 1
        best_s[...] = jnp.full(best_s.shape, -jnp.inf, f32)
        bidx_s[...] = jnp.zeros_like(bidx_s)

        for t in (1, 0, 2):
            proj_store(0, t, proj_half(0, t, 0) + proj_half(0, t, 1))

        def head_body(a, c):
            n = a * HEAD_U
            for n0 in range(0, G, HEAD_U):
                @pl.when(first & (n == n0))
                def _():
                    for g in range(n0 + 1, min(n0 + 1 + HEAD_U, G)):
                        wqkv_wait(g)
                    for g in range(n0 + 1 + HEAD_U, min(n0 + 1 + 2 * HEAD_U, G)):
                        for c in wqkv_in(g):
                            c.start()
                    if n0 == 0:
                        x_in(1).wait()
                        x_in(2).start()
                    if n0 <= 2 * G - LEAD < n0 + HEAD_U:
                        x_in(2).wait()
                    if n0 == G - HEAD_U:
                        wo_in.start()
                        for b in range(3, NB):
                            x_in(b).start()

            steps(n, [PLAN_HEAD] * HEAD_U, first_block=True)
            return c
        lax.fori_loop(0, G // HEAD_U, head_body, 0)

        @pl.when(first)
        def _():
            wo_in.wait()
            for b in range(3, NB):
                x_in(b).wait()
            for c in ffn_in:
                c.start()

        def body(a, c):
            n = a * BODY_U
            for b in range(NB - 2):
                @pl.when(last & (n == G * (b + 2)))
                def _():
                    x_out(b).start()

            steps(n, [PLAN_BODY] * BODY_U)
            return c
        lax.fori_loop(G // BODY_U, NSTEP // BODY_U - 1, body, 0)

        @pl.when(first)
        def _():
            for c in ffn_in:
                c.wait()

        steps(NSTEP - BODY_U, [PLAN_BODY] * (BODY_U - 1) + [PLAN_LAST])

        @pl.when(last)
        def _():
            for b in range(NB - 2, NB):
                x_out(b).start()

        best = best_s[...]
        top = jnp.max(best, axis=0, keepdims=True)
        idx = jnp.clip(jnp.min(jnp.where(best == top, bidx_s[...], S)), 0, S - 1)
        slab = rows_of(idx // 16, 16)
        sel = lax.broadcasted_iota(i32, (16, D), 0) == idx % 16
        hs = h1_s[slab, :]
        gate = _dot(hs, wg_s[...])
        up = _dot(hs, wu_s[...])
        y = _dot((gate * jax.nn.sigmoid(gate) * up).astype(bf16), wd_s[:, 0:D])
        y = y * jax.nn.sigmoid(top[:, 0:1])

        @pl.when(last)
        def _():
            for b in range(NB):
                x_out(b).wait()

        xs = x_s[slab, :].astype(f32)
        xs = jnp.where(sel, xs + y, xs).astype(bf16)
        x_s[slab, :] = xs

        @pl.when(last)
        def _():
            c = pltpu.make_async_copy(x_s.at[slab], out_hbm.at[slab], sem_o.at[0])
            c.start()
            c.wait()

        h_s[slab, :] = _ln(xs.astype(f32)).astype(bf16)
        return carry

    lax.fori_loop(0, LAYERS, layer, 0)


@jax.jit
def pallas_interleave_layers__sliding_block__moe_arch_mod__prompt_kernel(
    A_x: jax.Array,
    A_wqkv: jax.Array,
    A_wo: jax.Array,
    B_x: jax.Array,
    B_w_r: jax.Array,
    B_w_gate: jax.Array,
    B_w_up: jax.Array,
    B_w_down: jax.Array,
):
    del B_x
    hbm = pl.BlockSpec(memory_space=pl.ANY)
    out = pl.pallas_call(
        _kernel,
        in_specs=[hbm, hbm, hbm, pl.BlockSpec(memory_space=pltpu.VMEM), hbm, hbm, hbm],
        out_specs=hbm,
        out_shape=jax.ShapeDtypeStruct((S, D), bf16),
        scratch_shapes=[
            pltpu.VMEM((S, D), bf16),
            pltpu.VMEM((S, D), bf16),
            pltpu.VMEM((S, D), bf16),
            pltpu.VMEM((2, R, 128), bf16),
            pltpu.VMEM((G, S, 128), bf16),
            pltpu.VMEM((G, S // 128, 128, 128), bf16),
            pltpu.VMEM((G, S, 128), bf16),
            pltpu.VMEM((G, 3, D, 128), bf16),
            pltpu.VMEM((D, D + 128), bf16),
            pltpu.VMEM((D, F), bf16),
            pltpu.VMEM((D, F), bf16),
            pltpu.VMEM((F, D + 128), bf16),
            pltpu.VMEM((8, 128), f32),
            pltpu.VMEM((8, 128), i32),
            pltpu.VMEM((8, 128), u32),
            pltpu.VMEM((8, D), f32),
            pltpu.SemaphoreType.DMA((NB,)),
            pltpu.SemaphoreType.DMA((G + 4,)),
            pltpu.SemaphoreType.DMA((NB,)),
        ],
        compiler_params=pltpu.CompilerParams(vmem_limit_bytes=100 * 1024 * 1024),
    )(A_x.reshape(S, D), A_wqkv, A_wo, B_w_r,
      B_w_gate, B_w_up, B_w_down)
    return out.reshape(1, S, D)
```

```python
import math

import jax
import jax.numpy as jnp
from jax import lax
import jax.experimental.pallas as pl
import jax.experimental.pallas.tpu as pltpu

S, D, F = 2048, 1024, 3584
DH = 32
HPG = 4
G = D // 128
R = 512
NQ = R // 128
NB = S // R
PR = R // G
NP = S // PR
NSTEP = NB * G
LAYERS = 2
EPS = 1e-5
WIN = 256
NW = WIN // DH
PACE, PFRAC = 4, 0.7
LG = 99
XB = 4
HEAD_U, BODY_U = 2, 1
HS = 1
TB = 2
GATE, SGATE = 448, 1
PLAN_HEAD = "V0 s1 Q0 e1 p1 s2 V1 e2 p2 s0 Q1 e0 p0 N0 s3 K0 e3 p3 K1"
PLAN_BODY = "N0 o0 s0 V0 e0 p0 s1 V1 e1 p1 s2 K0 e2 o1 Q0 p2 s3 K1 e3 p3 Q1"
PLAN_LAST = ("N0 o0 s0 o1 e0 p0 s1 o2 e1 o3 p1 s2 o4 e2 o5 p2 s3 o6 e3 o7 p3 "
             "o8 o9 o10 o11 o12 o13 o14 o15 o16 o17")
LEAD = G + 1
QSCALE = DH ** -0.5 * math.log2(math.e)

bf16 = jnp.bfloat16
f32 = jnp.float32
u32 = jnp.uint32
i32 = jnp.int32


def _ln(x):
    m = jnp.mean(x, axis=-1, keepdims=True)
    xc = x - m
    v = jnp.mean(xc * xc, axis=-1, keepdims=True)
    return xc * lax.rsqrt(v + EPS)


def _dot(a, b):
    return jnp.dot(a, b, preferred_element_type=f32)


def _kernel(x_hbm, wqkv_hbm, wo_hbm, wr_ref, wg_hbm, wu_hbm, wd_hbm, out_hbm,
            x_s, h_s, h1_s, q_s, k_s, vt_s, o_s, wqkv_s, wo_s, wg_s, wu_s, wd_s,
            best_s, bidx_s, zero_s, wr_s, sem_x, sem_w, sem_o):

    def x_in(b):
        edges = (0, LEAD * PR, (LEAD + HEAD_U) * PR, S)
        rows = pl.ds(edges[b], edges[b + 1] - edges[b])
        return pltpu.make_async_copy(x_hbm.at[rows], x_s.at[rows], sem_x.at[b])

    def wqkv_in(g):
        return [pltpu.make_async_copy(
            wqkv_hbm.at[:, pl.ds(t * D + g * 128, 128)], wqkv_s.at[g, t], sem_w.at[g])
            for t in range(3)]

    def wqkv_wait(g):
        pltpu.make_async_copy(wqkv_s.at[g], wqkv_s.at[g], sem_w.at[g]).wait()

    wo_in = pltpu.make_async_copy(wo_hbm, wo_s.at[:, 0:D], sem_w.at[G])
    ffn_in = [pltpu.make_async_copy(a, b, sem_w.at[G + 1 + i]) for i, (a, b) in
              enumerate(((wg_hbm, wg_s), (wu_hbm, wu_s), (wd_hbm, wd_s.at[:, 0:D])))]

    def x_out(b):
        rows = pl.ds(b * R, R)
        return pltpu.make_async_copy(x_s.at[rows], out_hbm.at[rows], sem_o.at[b])

    x_in(0).start()
    wr_s[...] = jnp.broadcast_to(wr_ref[...].astype(f32).reshape(1, D), (8, D))
    zero_s[...] = jnp.zeros_like(zero_s)

    def rows_of(p, n):
        return pl.ds(p * n if isinstance(p, int) else pl.multiple_of(p * n, n), n)

    def ln_load(p):
        return x_s[rows_of(p, PR), :].astype(f32)

    def ln_store(x, p):
        h_s[rows_of(p, PR), :] = _ln(x).astype(bf16)

    def epilogue(y, p):
        x1 = ln_load(p) + y
        xc = x1 - jnp.mean(x1, axis=-1, keepdims=True)
        rstd = lax.rsqrt(jnp.mean(xc * xc, axis=-1, keepdims=True) + EPS)
        r = jnp.sum(xc * wr_s[0:1, :], axis=-1, keepdims=True) * rstd
        h1 = xc * rstd
        xb = (x1 + h1).astype(bf16)
        x_s[rows_of(p, PR), :] = xb
        h1_s[rows_of(p, PR), :] = h1.astype(bf16)
        r = jnp.broadcast_to(r, (PR, 128))
        best, bidx = best_s[...], bidx_s[...]
        row = lax.broadcasted_iota(i32, (8, 128), 0) + p * PR
        for t in range(PR // 8):
            rt = r[t * 8:(t + 1) * 8]
            up = rt > best
            best = jnp.where(up, rt, best)
            bidx = jnp.where(up, row + t * 8, bidx)
        best_s[...] = best
        bidx_s[...] = bidx
        return [bidx] + [xb[:r] for r in range(16, PR + 1, 16)][:XB]

    def proj_half(n, t, half, tok=None):
        i, g = n // G, n % G
        ks = pl.ds(half * (D // 2), D // 2)
        h = h_s[rows_of(i, R), ks]
        if tok is not None:
            x = pltpu.bitcast(h[GATE:GATE + 16], u32) | jnp.concatenate([tok] * (D // 256), axis=1)
            h = jnp.concatenate([h[:GATE], pltpu.bitcast(x, bf16), h[GATE + 16:]], axis=0)
        return _dot(h, wqkv_s[g, t, ks, :])

    def proj_store(n, t, y):
        i, g = n // G, n % G
        done = []
        if t == 0:
            q_s[n % 2] = (y * QSCALE).astype(bf16)
        elif t == 1:
            k_s[g, rows_of(i, R), :] = y.astype(bf16)
        else:
            for j in range(NQ):
                yt = y[j * 128:(j + 1) * 128]
                yt = yt.astype(bf16).T if TB > 1 else yt.T.astype(bf16)
                vt_s[g, i * NQ + j] = yt
                done.append(yt)
        return done

    def o_load(p):
        return jnp.concatenate([o_s[g, rows_of(p, PR), :] for g in range(G)], axis=1)

    def oproj_half(o, half):
        return _dot(o, wo_s[:, pl.ds(half * (D // 2), D // 2)])

    def shift_sel(bit, hi, lo):
        if hi is None and lo is None:
            return None
        ref = lo if hi is None else hi
        lane = lax.broadcasted_iota(i32, ref.shape, 1)
        zero = jnp.zeros_like(ref)
        return jnp.where(lane & (DH * bit) != 0, zero if hi is None else hi,
                         zero if lo is None else lo)

    def lane_rolls(x):
        x = pltpu.bitcast(x, u32)
        return [x] + [pltpu.roll(x, DH * s, 1) for s in range(1, HPG)]

    def attn_load(n, first_block):
        i, g = n // G, n % G
        back = 0 if first_block else WIN // 128
        qr = lane_rolls(q_s[n % 2])
        kr = lane_rolls(k_s[g, pl.ds(pl.multiple_of(i * R - back * 128, 128), R + back * 128), :])
        vt = {t: vt_s[g, i * NQ + t] for t in range(-back, NQ)}
        lo = -back * HPG
        kc = [{c + lo: x[c * 16:(c + 1) * 16] for c in range(x.shape[0] // 16)} for x in kr]
        u = [{c: shift_sel(1, kc[(s + 1) % HPG].get(c + 1), kc[s].get(c))
              for c in range(-NW, R // DH - 1)} for s in range(HPG)]
        ks = [{c: shift_sel(2, u[(2 - h) % HPG][c + 2], u[-h % HPG][c])
               for c in range(-NW, R // DH - 3)} for h in range(HPG)]
        return qr, ks, vt

    def qk(qr, ks, j, h, chunks, tok):
        w = []
        for a in range(HPG):
            x = qr[(a - h) % HPG][j * 64 + a * 16:j * 64 + (a + 1) * 16]
            lane = lax.broadcasted_iota(i32, x.shape, 1)
            w.append(jnp.where(lane // DH == a, x, jnp.zeros_like(x)))
        if tok is not None:
            w[0] = w[0] | jnp.concatenate([tok] * 2, axis=0)
        w = pltpu.bitcast(jnp.concatenate(w, axis=0), bf16)
        k = pltpu.bitcast(jnp.concatenate([ks[h][j * HPG - NW + c] for c in chunks], axis=0), bf16)
        s = lax.dot_general(k, w, (((1,), (1,)), ((), ())), preferred_element_type=f32)
        return {c: s[a * DH:(a + 1) * DH] for a, c in enumerate(chunks)}

    def softmax(ss, start, pace, zv):
        lane = lax.broadcasted_iota(i32, (DH, 128), 1)
        tri = lax.broadcasted_iota(i32, (DH, 128), 0) <= lane % DH
        wrap = 0 in ss[0]
        ms = []
        for s in ss:
            s[NW] = jnp.where(tri, s[NW], s.pop(0) if wrap else -jnp.inf)
            m = None
            for c in s:
                if c < start:
                    s[c] = jnp.where(lane // DH >= start - c, s[c], -jnp.inf)
                d = jnp.max(s[c].reshape(DH // 8, 8, 128), axis=0)
                m = d if m is None else jnp.maximum(m, d)
            ms.append(jnp.broadcast_to(jnp.max(m, axis=0, keepdims=True), (8, 128)))
        ls, es, mp = [None] * len(ss), [{} for _ in ss], list(ms)
        for a, c in enumerate(ss[0]):
            for h, s in enumerate(ss):
                if pace is not None and a % PACE == 0:
                    pr = pace.shape[0]
                    r0 = int((a + HS * PACE * h / len(ss)) * pace.size // 128 * PFRAC) // len(s) // 8 * 8
                    src = pace[r0 % pr:r0 % pr + 8, r0 // pr * 128:(r0 // pr + 1) * 128]
                    mp[h] = pltpu.bitcast(
                        pltpu.bitcast(ms[h], u32) | (pltpu.bitcast(src, u32) & zv), f32)
                x = jnp.exp2(s[c].reshape(DH // 8, 8, 128) - mp[h])
                t = jnp.sum(x, axis=0)
                ls[h] = t if ls[h] is None else ls[h] + t
                es[h][c] = x.reshape(DH, 128)
        out = []
        for e, l in zip(es, ls):
            if wrap:
                x = e[NW]
                e[NW] = jnp.where(tri, x, 0.0)
                e[0] = x - e[NW]
            t = {c: shift_sel(1, e.get(c - 1), e.get(c)) for c in range(NW + 2)}
            p = {c: shift_sel(2, t.get(c - 2), t.get(c)) for c in range(max(start, 0), NW + HPG)}
            p = {c // HPG - WIN // 128: jnp.concatenate([p[c + a] for a in range(HPG)], axis=0)
                 for c in range(max(start, 0), NW + HPG, HPG)}
            out.append((p, jnp.sum(l, axis=0, keepdims=True)))
        return out

    def steps(n0, plans, first_block=False):
        pn = [(n0 + LEAD + a) % NP for a in range(len(plans))]
        xl = [ln_load(p) if "N" in plan else None for p, plan in zip(pn, plans)]
        oi = [o_load(n0 - G + a) if "o" in plan else None for a, plan in enumerate(plans)]
        due = []
        for a, plan in enumerate(plans):
            step(n0 + a, plan, first_block, xl[a], pn[a], oi[a], due)

    def step(n, plan, first_block, xl, pn, oi, due):
        zv = zero_s[...]
        qr, ks, vt = attn_load(n, first_block)
        part, ss, sm = {}, {}, {}
        pace = None

        def settle():
            now = [x for wait, x in due if wait == 0]
            due[:] = [(wait - 1, x) for wait, x in due if wait]
            tok = zv if now else None
            for x in now:
                tok = tok & pltpu.bitcast(x[-32 // x.dtype.itemsize:, -128:], u32)
            return tok

        for op in plan.split():
            kind, j = op[0], int(op[1:])
            start = NW - j * HPG if first_block else 0
            if kind == "o":
                piece = n - G + j // 2
                if j > 1 and j % 2 == 0:
                    oi = o_load(piece)
                pace = oproj_half(oi, j % 2)
                if j % 2:
                    done = epilogue(jnp.concatenate([part["o"], pace], axis=1), piece)
                    due.extend((LG, x) for x in done)
                part["o"] = pace
            elif kind == "N":
                ln_store(xl, pn)
            elif kind in "QKV":
                t = "QKV".index(kind)
                pace = proj_half(n + 1, t, j, settle())
                if j:
                    due.extend((0, x) for x in proj_store(n + 1, t, part[t] + pace))
                part[t] = pace
            elif kind == "s":
                chunks = ([0] if start <= 0 else []) + [NW]
                chunks += range(max(start - HPG + 1, 1), NW)
                tok = None
                if SGATE and pace is not None:
                    tok = pltpu.bitcast(pace[0:8, 0:128], u32) & zv
                ss[j] = [qk(qr, ks, j, h, chunks, tok) for h in range(HPG)]
                pace = None
            elif kind == "e":
                sm[j] = softmax(ss[j], start, pace, zv)
            else:
                ot = [None] * HPG
                for t in sm[j][0][0]:
                    for h, (p, _) in enumerate(sm[j]):
                        y = _dot(vt[j + t][h * DH:(h + 1) * DH], p[t].astype(bf16))
                        ot[h] = y if ot[h] is None else ot[h] + y
                ot = jnp.concatenate([y * (1.0 / l) for y, (_, l) in zip(ot, sm[j])], axis=0)
                ot = ot.astype(bf16).T if TB else ot.T.astype(bf16)
                o_s[n % G, rows_of((n // G) * NQ + j, 128), :] = ot
                due.append((0, ot))


    x_in(0).wait()
    for c in wqkv_in(0):
        c.start()

    def ln_head(p, c):
        ln_store(ln_load(p), p)
        return c
    lax.fori_loop(0, LEAD, ln_head, 0, unroll=3)
    x_in(1).start()
    for g in range(1, 1 + HEAD_U):
        for c in wqkv_in(g):
            c.start()
    wqkv_wait(0)

    def layer(li, carry):
        first, last = li == 0, li == LAYERS - 1
        best_s[...] = jnp.full(best_s.shape, -jnp.inf, f32)
        bidx_s[...] = jnp.zeros_like(bidx_s)

        for t in (1, 0, 2):
            proj_store(0, t, proj_half(0, t, 0) + proj_half(0, t, 1))

        def head_body(a, c):
            n = a * HEAD_U
            for n0 in range(0, G, HEAD_U):
                @pl.when(first & (n == n0))
                def _():
                    for g in range(n0 + 1, min(n0 + 1 + HEAD_U, G)):
                        wqkv_wait(g)
                    for g in range(n0 + 1 + HEAD_U, min(n0 + 1 + 2 * HEAD_U, G)):
                        for c in wqkv_in(g):
                            c.start()
                    if n0 == 0:
                        x_in(1).wait()
                        x_in(2).start()
                    if n0 == HEAD_U:
                        x_in(2).wait()
                        wo_in.start()

            steps(n, [PLAN_HEAD] * HEAD_U, first_block=True)
            return c
        lax.fori_loop(0, G // HEAD_U, head_body, 0)

        @pl.when(first)
        def _():
            wo_in.wait()
            for c in ffn_in:
                c.start()

        def body(a, c):
            n = a * BODY_U
            for b in range(NB - 2):
                @pl.when(last & (n == G * (b + 2)))
                def _():
                    x_out(b).start()

            steps(n, [PLAN_BODY] * BODY_U)
            return c
        lax.fori_loop(G // BODY_U, NSTEP // BODY_U - 1, body, 0)

        @pl.when(first)
        def _():
            for c in ffn_in:
                c.wait()

        steps(NSTEP - BODY_U, [PLAN_BODY] * (BODY_U - 1) + [PLAN_LAST])

        @pl.when(last)
        def _():
            for b in range(NB - 2, NB):
                x_out(b).start()

        best = best_s[...]
        top = jnp.max(best, axis=0, keepdims=True)
        idx = jnp.clip(jnp.min(jnp.where(best == top, bidx_s[...], S)), 0, S - 1)
        slab = rows_of(idx // 16, 16)
        sel = lax.broadcasted_iota(i32, (16, D), 0) == idx % 16
        hs = h1_s[slab, :]
        gate = _dot(hs, wg_s[...])
        up = _dot(hs, wu_s[...])
        y = _dot((gate * jax.nn.sigmoid(gate) * up).astype(bf16), wd_s[:, 0:D])
        y = y * jax.nn.sigmoid(top[:, 0:1])

        @pl.when(last)
        def _():
            for b in range(NB):
                x_out(b).wait()

        xs = x_s[slab, :].astype(f32)
        xs = jnp.where(sel, xs + y, xs).astype(bf16)
        x_s[slab, :] = xs

        @pl.when(last)
        def _():
            c = pltpu.make_async_copy(x_s.at[slab], out_hbm.at[slab], sem_o.at[0])
            c.start()
            c.wait()

        h_s[slab, :] = _ln(xs.astype(f32)).astype(bf16)
        return carry

    lax.fori_loop(0, LAYERS, layer, 0)


@jax.jit
def pallas_interleave_layers__sliding_block__moe_arch_mod__prompt_kernel(
    A_x: jax.Array,
    A_wqkv: jax.Array,
    A_wo: jax.Array,
    B_x: jax.Array,
    B_w_r: jax.Array,
    B_w_gate: jax.Array,
    B_w_up: jax.Array,
    B_w_down: jax.Array,
):
    del B_x
    hbm = pl.BlockSpec(memory_space=pl.ANY)
    out = pl.pallas_call(
        _kernel,
        in_specs=[hbm, hbm, hbm, pl.BlockSpec(memory_space=pltpu.VMEM), hbm, hbm, hbm],
        out_specs=hbm,
        out_shape=jax.ShapeDtypeStruct((S, D), bf16),
        scratch_shapes=[
            pltpu.VMEM((S, D), bf16),
            pltpu.VMEM((S, D), bf16),
            pltpu.VMEM((S, D), bf16),
            pltpu.VMEM((2, R, 128), bf16),
            pltpu.VMEM((G, S, 128), bf16),
            pltpu.VMEM((G, S // 128, 128, 128), bf16),
            pltpu.VMEM((G, S, 128), bf16),
            pltpu.VMEM((G, 3, D, 128), bf16),
            pltpu.VMEM((D, D + 128), bf16),
            pltpu.VMEM((D, F), bf16),
            pltpu.VMEM((D, F), bf16),
            pltpu.VMEM((F, D + 128), bf16),
            pltpu.VMEM((8, 128), f32),
            pltpu.VMEM((8, 128), i32),
            pltpu.VMEM((8, 128), u32),
            pltpu.VMEM((8, D), f32),
            pltpu.SemaphoreType.DMA((3,)),
            pltpu.SemaphoreType.DMA((G + 4,)),
            pltpu.SemaphoreType.DMA((NB,)),
        ],
        compiler_params=pltpu.CompilerParams(vmem_limit_bytes=100 * 1024 * 1024),
    )(A_x.reshape(S, D), A_wqkv, A_wo, B_w_r,
      B_w_gate, B_w_up, B_w_down)
    return out.reshape(1, S, D)
```

```python
import math

import jax
import jax.numpy as jnp
from jax import lax
import jax.experimental.pallas as pl
import jax.experimental.pallas.tpu as pltpu

S, D, F = 2048, 1024, 3584
DH = 32
HPG = 4
G = D // 128
R = 512
NQ = R // 128
NB = S // R
PR = R // G
NP = S // PR
NSTEP = NB * G
LAYERS = 2
EPS = 1e-5
WIN = 256
NW = WIN // DH
PACE, PFRAC = 4, 0.65
LG = 3
XB = 4
HEAD_U, BODY_U = 2, 2
HS = 1
TB = 2
GATE, SGATE = 416, 1
PLAN_HEAD = "V0 s1 Q0 e1 p1 s2 V1 e2 p2 s0 Q1 e0 p0 N0 s3 K0 e3 p3 K1"
PLAN_BODY = "o0 N0 o1 s0 V0 e0 p0 Q0 s1 K0 e1 p1 s2 K1 e2 p2 s3 V1 e3 p3 Q1"
PLAN_LAST = ("N0 o0 s0 o1 e0 p0 s1 o2 e1 o3 p1 s2 o4 e2 o5 p2 s3 o6 e3 o7 p3 "
             "o8 o9 o10 o11 o12 o13 o14 o15 o16 o17")
LEAD = G + 1
QSCALE = DH ** -0.5 * math.log2(math.e)

bf16 = jnp.bfloat16
f32 = jnp.float32
u32 = jnp.uint32
i32 = jnp.int32


def _ln(x):
    m = jnp.mean(x, axis=-1, keepdims=True)
    xc = x - m
    v = jnp.mean(xc * xc, axis=-1, keepdims=True)
    return xc * lax.rsqrt(v + EPS)


def _dot(a, b):
    return jnp.dot(a, b, preferred_element_type=f32)


def _kernel(x_hbm, wqkv_hbm, wo_hbm, wr_ref, wg_hbm, wu_hbm, wd_hbm, out_hbm,
            x_s, h_s, h1_s, q_s, k_s, vt_s, o_s, wqkv_s, wo_s, wg_s, wu_s, wd_s,
            best_s, bidx_s, zero_s, wr_s, sem_x, sem_w, sem_o):

    def x_in(b):
        edges = (0, LEAD * PR, (LEAD + HEAD_U) * PR, S)
        rows = pl.ds(edges[b], edges[b + 1] - edges[b])
        return pltpu.make_async_copy(x_hbm.at[rows], x_s.at[rows], sem_x.at[b])

    def wqkv_in(g):
        return [pltpu.make_async_copy(
            wqkv_hbm.at[:, pl.ds(t * D + g * 128, 128)], wqkv_s.at[g, t], sem_w.at[g])
            for t in range(3)]

    def wqkv_wait(g):
        pltpu.make_async_copy(wqkv_s.at[g], wqkv_s.at[g], sem_w.at[g]).wait()

    wo_in = pltpu.make_async_copy(wo_hbm, wo_s.at[:, 0:D], sem_w.at[G])
    ffn_in = [pltpu.make_async_copy(a, b, sem_w.at[G + 1 + i]) for i, (a, b) in
              enumerate(((wg_hbm, wg_s), (wu_hbm, wu_s), (wd_hbm, wd_s.at[:, 0:D])))]

    def x_out(b):
        rows = pl.ds(b * R, R)
        return pltpu.make_async_copy(x_s.at[rows], out_hbm.at[rows], sem_o.at[b])

    x_in(0).start()
    wr_s[...] = jnp.broadcast_to(wr_ref[...].astype(f32).reshape(1, D), (8, D))
    zero_s[...] = jnp.zeros_like(zero_s)

    def rows_of(p, n):
        return pl.ds(p * n if isinstance(p, int) else pl.multiple_of(p * n, n), n)

    def ln_load(p):
        return x_s[rows_of(p, PR), :].astype(f32)

    def ln_store(x, p):
        h_s[rows_of(p, PR), :] = _ln(x).astype(bf16)

    def epilogue(y, p):
        x1 = ln_load(p) + y
        xc = x1 - jnp.mean(x1, axis=-1, keepdims=True)
        rstd = lax.rsqrt(jnp.mean(xc * xc, axis=-1, keepdims=True) + EPS)
        r = jnp.sum(xc * wr_s[0:1, :], axis=-1, keepdims=True) * rstd
        h1 = xc * rstd
        xb = (x1 + h1).astype(bf16)
        x_s[rows_of(p, PR), :] = xb
        h1_s[rows_of(p, PR), :] = h1.astype(bf16)
        r = jnp.broadcast_to(r, (PR, 128))
        best, bidx = best_s[...], bidx_s[...]
        row = lax.broadcasted_iota(i32, (8, 128), 0) + p * PR
        for t in range(PR // 8):
            rt = r[t * 8:(t + 1) * 8]
            up = rt > best
            best = jnp.where(up, rt, best)
            bidx = jnp.where(up, row + t * 8, bidx)
        best_s[...] = best
        bidx_s[...] = bidx
        return [bidx] + [xb[:r] for r in range(16, PR + 1, 16)][:XB]

    def proj_half(n, t, half, tok=None):
        i, g = n // G, n % G
        ks = pl.ds(half * (D // 2), D // 2)
        h = h_s[rows_of(i, R), ks]
        if tok is not None:
            x = pltpu.bitcast(h[GATE:GATE + 16], u32) | jnp.concatenate([tok] * (D // 256), axis=1)
            h = jnp.concatenate([h[:GATE], pltpu.bitcast(x, bf16), h[GATE + 16:]], axis=0)
        return _dot(h, wqkv_s[g, t, ks, :])

    def proj_store(n, t, y):
        i, g = n // G, n % G
        done = []
        if t == 0:
            q_s[n % 2] = (y * QSCALE).astype(bf16)
        elif t == 1:
            k_s[g, rows_of(i, R), :] = y.astype(bf16)
        else:
            for j in range(NQ):
                yt = y[j * 128:(j + 1) * 128]
                yt = yt.astype(bf16).T if TB > 1 else yt.T.astype(bf16)
                vt_s[g, i * NQ + j] = yt
                done.append(yt)
        return done

    def o_load(p):
        return jnp.concatenate([o_s[g, rows_of(p, PR), :] for g in range(G)], axis=1)

    def oproj_half(o, half):
        return _dot(o, wo_s[:, pl.ds(half * (D // 2), D // 2)])

    def shift_sel(bit, hi, lo):
        if hi is None and lo is None:
            return None
        ref = lo if hi is None else hi
        lane = lax.broadcasted_iota(i32, ref.shape, 1)
        zero = jnp.zeros_like(ref)
        return jnp.where(lane & (DH * bit) != 0, zero if hi is None else hi,
                         zero if lo is None else lo)

    def lane_rolls(x):
        x = pltpu.bitcast(x, u32)
        return [x] + [pltpu.roll(x, DH * s, 1) for s in range(1, HPG)]

    def attn_load(n, first_block):
        i, g = n // G, n % G
        back = 0 if first_block else WIN // 128
        qr = lane_rolls(q_s[n % 2])
        kr = lane_rolls(k_s[g, pl.ds(pl.multiple_of(i * R - back * 128, 128), R + back * 128), :])
        vt = {t: vt_s[g, i * NQ + t] for t in range(-back, NQ)}
        lo = -back * HPG
        kc = [{c + lo: x[c * 16:(c + 1) * 16] for c in range(x.shape[0] // 16)} for x in kr]
        u = [{c: shift_sel(1, kc[(s + 1) % HPG].get(c + 1), kc[s].get(c))
              for c in range(-NW, R // DH - 1)} for s in range(HPG)]
        ks = [{c: shift_sel(2, u[(2 - h) % HPG][c + 2], u[-h % HPG][c])
               for c in range(-NW, R // DH - 3)} for h in range(HPG)]
        return qr, ks, vt

    def qk(qr, ks, j, h, chunks, tok):
        w = []
        for a in range(HPG):
            x = qr[(a - h) % HPG][j * 64 + a * 16:j * 64 + (a + 1) * 16]
            lane = lax.broadcasted_iota(i32, x.shape, 1)
            w.append(jnp.where(lane // DH == a, x, jnp.zeros_like(x)))
        if tok is not None:
            w[0] = w[0] | jnp.concatenate([tok] * 2, axis=0)
        w = pltpu.bitcast(jnp.concatenate(w, axis=0), bf16)
        k = pltpu.bitcast(jnp.concatenate([ks[h][j * HPG - NW + c] for c in chunks], axis=0), bf16)
        s = lax.dot_general(k, w, (((1,), (1,)), ((), ())), preferred_element_type=f32)
        return {c: s[a * DH:(a + 1) * DH] for a, c in enumerate(chunks)}

    def softmax(ss, start, pace, zv):
        lane = lax.broadcasted_iota(i32, (DH, 128), 1)
        tri = lax.broadcasted_iota(i32, (DH, 128), 0) <= lane % DH
        wrap = 0 in ss[0]
        ms = []
        for s in ss:
            s[NW] = jnp.where(tri, s[NW], s.pop(0) if wrap else -jnp.inf)
            m = None
            for c in s:
                if c < start:
                    s[c] = jnp.where(lane // DH >= start - c, s[c], -jnp.inf)
                d = jnp.max(s[c].reshape(DH // 8, 8, 128), axis=0)
                m = d if m is None else jnp.maximum(m, d)
            ms.append(jnp.broadcast_to(jnp.max(m, axis=0, keepdims=True), (8, 128)))
        ls, es, mp = [None] * len(ss), [{} for _ in ss], list(ms)
        for a, c in enumerate(ss[0]):
            for h, s in enumerate(ss):
                if pace is not None and a % PACE == 0:
                    pr = pace.shape[0]
                    r0 = int((a + HS * PACE * h / len(ss)) * pace.size // 128 * PFRAC) // len(s) // 8 * 8
                    src = pace[r0 % pr:r0 % pr + 8, r0 // pr * 128:(r0 // pr + 1) * 128]
                    mp[h] = pltpu.bitcast(
                        pltpu.bitcast(ms[h], u32) | (pltpu.bitcast(src, u32) & zv), f32)
                x = jnp.exp2(s[c].reshape(DH // 8, 8, 128) - mp[h])
                t = jnp.sum(x, axis=0)
                ls[h] = t if ls[h] is None else ls[h] + t
                es[h][c] = x.reshape(DH, 128)
        out = []
        for e, l in zip(es, ls):
            if wrap:
                x = e[NW]
                e[NW] = jnp.where(tri, x, 0.0)
                e[0] = x - e[NW]
            t = {c: shift_sel(1, e.get(c - 1), e.get(c)) for c in range(NW + 2)}
            p = {c: shift_sel(2, t.get(c - 2), t.get(c)) for c in range(max(start, 0), NW + HPG)}
            p = {c // HPG - WIN // 128: jnp.concatenate([p[c + a] for a in range(HPG)], axis=0)
                 for c in range(max(start, 0), NW + HPG, HPG)}
            out.append((p, jnp.sum(l, axis=0, keepdims=True)))
        return out

    def steps(n0, plans, first_block=False):
        pn = [(n0 + LEAD + a) % NP for a in range(len(plans))]
        xl = [ln_load(p) if "N" in plan else None for p, plan in zip(pn, plans)]
        oi = [o_load(n0 - G + a) if "o" in plan else None for a, plan in enumerate(plans)]
        due = []
        for a, plan in enumerate(plans):
            step(n0 + a, plan, first_block, xl[a], pn[a], oi[a], due)

    def step(n, plan, first_block, xl, pn, oi, due):
        zv = zero_s[...]
        qr, ks, vt = attn_load(n, first_block)
        part, ss, sm = {}, {}, {}
        pace = None

        def settle():
            now = [x for wait, x in due if wait == 0]
            due[:] = [(wait - 1, x) for wait, x in due if wait]
            tok = zv if now else None
            for x in now:
                tok = tok & pltpu.bitcast(x[-32 // x.dtype.itemsize:, -128:], u32)
            return tok

        for op in plan.split():
            kind, j = op[0], int(op[1:])
            start = NW - j * HPG if first_block else 0
            if kind == "o":
                piece = n - G + j // 2
                if j > 1 and j % 2 == 0:
                    oi = o_load(piece)
                pace = oproj_half(oi, j % 2)
                if j % 2:
                    done = epilogue(jnp.concatenate([part["o"], pace], axis=1), piece)
                    due.extend((LG, x) for x in done)
                part["o"] = pace
            elif kind == "N":
                ln_store(xl, pn)
            elif kind in "QKV":
                t = "QKV".index(kind)
                pace = proj_half(n + 1, t, j, settle())
                if j:
                    due.extend((0, x) for x in proj_store(n + 1, t, part[t] + pace))
                part[t] = pace
            elif kind == "s":
                chunks = ([0] if start <= 0 else []) + [NW]
                chunks += range(max(start - HPG + 1, 1), NW)
                tok = None
                if SGATE and pace is not None:
                    tok = pltpu.bitcast(pace[0:8, 0:128], u32) & zv
                ss[j] = [qk(qr, ks, j, h, chunks, tok) for h in range(HPG)]
                pace = None
            elif kind == "e":
                sm[j] = softmax(ss[j], start, pace, zv)
            else:
                ot = [None] * HPG
                for t in sm[j][0][0]:
                    for h, (p, _) in enumerate(sm[j]):
                        y = _dot(vt[j + t][h * DH:(h + 1) * DH], p[t].astype(bf16))
                        ot[h] = y if ot[h] is None else ot[h] + y
                ot = jnp.concatenate([y * (1.0 / l) for y, (_, l) in zip(ot, sm[j])], axis=0)
                ot = ot.astype(bf16).T if TB else ot.T.astype(bf16)
                o_s[n % G, rows_of((n // G) * NQ + j, 128), :] = ot
                due.append((0, ot))


    x_in(0).wait()
    for c in wqkv_in(0):
        c.start()

    def ln_head(p, c):
        ln_store(ln_load(p), p)
        return c
    lax.fori_loop(0, LEAD, ln_head, 0, unroll=3)
    x_in(1).start()
    for g in range(1, 1 + HEAD_U):
        for c in wqkv_in(g):
            c.start()
    wqkv_wait(0)

    def layer(li, carry):
        first, last = li == 0, li == LAYERS - 1
        best_s[...] = jnp.full(best_s.shape, -jnp.inf, f32)
        bidx_s[...] = jnp.zeros_like(bidx_s)

        for t in (1, 0, 2):
            proj_store(0, t, proj_half(0, t, 0) + proj_half(0, t, 1))

        def head_body(a, c):
            n = a * HEAD_U
            for n0 in range(0, G, HEAD_U):
                @pl.when(first & (n == n0))
                def _():
                    for g in range(n0 + 1, min(n0 + 1 + HEAD_U, G)):
                        wqkv_wait(g)
                    for g in range(n0 + 1 + HEAD_U, min(n0 + 1 + 2 * HEAD_U, G)):
                        for c in wqkv_in(g):
                            c.start()
                    if n0 == 0:
                        x_in(1).wait()
                        x_in(2).start()
                    if n0 == HEAD_U:
                        x_in(2).wait()
                        wo_in.start()

            steps(n, [PLAN_HEAD] * HEAD_U, first_block=True)
            return c
        lax.fori_loop(0, G // HEAD_U, head_body, 0)

        @pl.when(first)
        def _():
            wo_in.wait()
            for c in ffn_in:
                c.start()

        def body(a, c):
            n = a * BODY_U
            for b in range(NB - 2):
                @pl.when(last & (n == G * (b + 2)))
                def _():
                    x_out(b).start()

            steps(n, [PLAN_BODY] * BODY_U)
            return c
        lax.fori_loop(G // BODY_U, NSTEP // BODY_U - 1, body, 0)

        @pl.when(first)
        def _():
            for c in ffn_in:
                c.wait()

        steps(NSTEP - BODY_U, [PLAN_BODY] * (BODY_U - 1) + [PLAN_LAST])

        @pl.when(last)
        def _():
            for b in range(NB - 2, NB):
                x_out(b).start()

        best = best_s[...]
        top = jnp.max(best, axis=0, keepdims=True)
        idx = jnp.clip(jnp.min(jnp.where(best == top, bidx_s[...], S)), 0, S - 1)
        slab = rows_of(idx // 16, 16)
        sel = lax.broadcasted_iota(i32, (16, D), 0) == idx % 16
        hs = h1_s[slab, :]
        gate = _dot(hs, wg_s[...])
        up = _dot(hs, wu_s[...])
        y = _dot((gate * jax.nn.sigmoid(gate) * up).astype(bf16), wd_s[:, 0:D])
        y = y * jax.nn.sigmoid(top[:, 0:1])

        @pl.when(last)
        def _():
            for b in range(NB):
                x_out(b).wait()

        xs = x_s[slab, :].astype(f32)
        xs = jnp.where(sel, xs + y, xs).astype(bf16)
        x_s[slab, :] = xs

        @pl.when(last)
        def _():
            c = pltpu.make_async_copy(x_s.at[slab], out_hbm.at[slab], sem_o.at[0])
            c.start()
            c.wait()

        h_s[slab, :] = _ln(xs.astype(f32)).astype(bf16)
        return carry

    lax.fori_loop(0, LAYERS, layer, 0)


@jax.jit
def pallas_interleave_layers__sliding_block__moe_arch_mod__prompt_kernel(
    A_x: jax.Array,
    A_wqkv: jax.Array,
    A_wo: jax.Array,
    B_x: jax.Array,
    B_w_r: jax.Array,
    B_w_gate: jax.Array,
    B_w_up: jax.Array,
    B_w_down: jax.Array,
):
    del B_x
    hbm = pl.BlockSpec(memory_space=pl.ANY)
    out = pl.pallas_call(
        _kernel,
        in_specs=[hbm, hbm, hbm, pl.BlockSpec(memory_space=pltpu.VMEM), hbm, hbm, hbm],
        out_specs=hbm,
        out_shape=jax.ShapeDtypeStruct((S, D), bf16),
        scratch_shapes=[
            pltpu.VMEM((S, D), bf16),
            pltpu.VMEM((S, D), bf16),
            pltpu.VMEM((S, D), bf16),
            pltpu.VMEM((2, R, 128), bf16),
            pltpu.VMEM((G, S, 128), bf16),
            pltpu.VMEM((G, S // 128, 128, 128), bf16),
            pltpu.VMEM((G, S, 128), bf16),
            pltpu.VMEM((G, 3, D, 128), bf16),
            pltpu.VMEM((D, D + 128), bf16),
            pltpu.VMEM((D, F), bf16),
            pltpu.VMEM((D, F), bf16),
            pltpu.VMEM((F, D + 128), bf16),
            pltpu.VMEM((8, 128), f32),
            pltpu.VMEM((8, 128), i32),
            pltpu.VMEM((8, 128), u32),
            pltpu.VMEM((8, D), f32),
            pltpu.SemaphoreType.DMA((3,)),
            pltpu.SemaphoreType.DMA((G + 4,)),
            pltpu.SemaphoreType.DMA((NB,)),
        ],
        compiler_params=pltpu.CompilerParams(vmem_limit_bytes=100 * 1024 * 1024),
    )(A_x.reshape(S, D), A_wqkv, A_wo, B_w_r,
      B_w_gate, B_w_up, B_w_down)
    return out.reshape(1, S, D)
```

```python
import math

import jax
import jax.numpy as jnp
from jax import lax
import jax.experimental.pallas as pl
import jax.experimental.pallas.tpu as pltpu

S, D, F = 2048, 1024, 3584
DH = 32
HPG = 4
G = D // 128
R = 512
NQ = R // 128
NB = S // R
PR = R // G
NP = S // PR
NSTEP = NB * G
LAYERS = 2
EPS = 1e-5
WIN = 256
NW = WIN // DH
HEAD_U, BODY_U = 2, 2
PACE, PFRAC = 4, 0.65
GATE = 416
EPI_WAIT = 3
PLAN_HEAD = "V0 s3 K0 e3 p3 s0 V1 e0 p0 N0 s2 Q0 e2 p2 s1 Q1 e1 p1 K1"
PLAN_BODY = "o0 N0 o1 s0 V0 e0 p0 Q0 s1 K0 e1 p1 s2 K1 e2 p2 s3 V1 e3 p3 Q1"
PLAN_LAST = ("N0 o0 s0 o1 e0 p0 s1 o2 e1 o3 p1 s2 o4 e2 o5 p2 s3 o6 e3 o7 p3 "
             "o8 o9 o10 o11 o12 o13 o14 o15 o16 o17")
LEAD = G + 1
QSCALE = DH ** -0.5 * math.log2(math.e)

bf16 = jnp.bfloat16
f32 = jnp.float32
u32 = jnp.uint32
i32 = jnp.int32


def _ln(x):
    m = jnp.mean(x, axis=-1, keepdims=True)
    xc = x - m
    v = jnp.mean(xc * xc, axis=-1, keepdims=True)
    return xc * lax.rsqrt(v + EPS)


def _dot(a, b):
    return jnp.dot(a, b, preferred_element_type=f32)


def _kernel(x_hbm, wqkv_hbm, wo_hbm, wr_ref, wg_hbm, wu_hbm, wd_hbm, out_hbm,
            x_s, h_s, h1_s, q_s, k_s, vt_s, o_s, wqkv_s, wo_s, wg_s, wu_s, wd_s,
            best_s, bidx_s, zero_s, wr_s, sem_x, sem_w, sem_o):

    def x_in(b):
        edges = (0, LEAD * PR, (LEAD + HEAD_U) * PR, S)
        rows = pl.ds(edges[b], edges[b + 1] - edges[b])
        return pltpu.make_async_copy(x_hbm.at[rows], x_s.at[rows], sem_x.at[b])

    def wqkv_in(g):
        return [pltpu.make_async_copy(
            wqkv_hbm.at[:, pl.ds(t * D + g * 128, 128)], wqkv_s.at[g, t], sem_w.at[g])
            for t in range(3)]

    def wqkv_wait(g):
        pltpu.make_async_copy(wqkv_s.at[g], wqkv_s.at[g], sem_w.at[g]).wait()

    wo_in = pltpu.make_async_copy(wo_hbm, wo_s.at[:, 0:D], sem_w.at[G])
    ffn_in = [pltpu.make_async_copy(a, b, sem_w.at[G + 1 + i]) for i, (a, b) in
              enumerate(((wg_hbm, wg_s), (wu_hbm, wu_s), (wd_hbm, wd_s.at[:, 0:D])))]

    def x_out(b):
        rows = pl.ds(b * R, R)
        return pltpu.make_async_copy(x_s.at[rows], out_hbm.at[rows], sem_o.at[b])

    x_in(0).start()
    wr_s[...] = jnp.broadcast_to(wr_ref[...].astype(f32).reshape(1, D), (8, D))
    zero_s[...] = jnp.zeros_like(zero_s)

    def rows_of(p, n):
        return pl.ds(p * n if isinstance(p, int) else pl.multiple_of(p * n, n), n)

    def ln_load(p):
        return x_s[rows_of(p, PR), :].astype(f32)

    def ln_store(x, p):
        h_s[rows_of(p, PR), :] = _ln(x).astype(bf16)

    def epilogue(y, p):
        x1 = ln_load(p) + y
        xc = x1 - jnp.mean(x1, axis=-1, keepdims=True)
        rstd = lax.rsqrt(jnp.mean(xc * xc, axis=-1, keepdims=True) + EPS)
        r = jnp.sum(xc * wr_s[0:1, :], axis=-1, keepdims=True) * rstd
        h1 = xc * rstd
        xb = (x1 + h1).astype(bf16)
        x_s[rows_of(p, PR), :] = xb
        h1_s[rows_of(p, PR), :] = h1.astype(bf16)
        r = jnp.broadcast_to(r, (PR, 128))
        best, bidx = best_s[...], bidx_s[...]
        row = lax.broadcasted_iota(i32, (8, 128), 0) + p * PR
        for t in range(PR // 8):
            rt = r[t * 8:(t + 1) * 8]
            up = rt > best
            best = jnp.where(up, rt, best)
            bidx = jnp.where(up, row + t * 8, bidx)
        best_s[...] = best
        bidx_s[...] = bidx
        return [bidx] + [xb[:r] for r in range(16, PR + 1, 16)]

    def proj_half(n, t, half, tok=None):
        i, g = n // G, n % G
        ks = pl.ds(half * (D // 2), D // 2)
        h = h_s[rows_of(i, R), ks]
        if tok is not None:
            x = pltpu.bitcast(h[GATE:GATE + 16], u32) | jnp.concatenate([tok] * (D // 256), axis=1)
            h = jnp.concatenate([h[:GATE], pltpu.bitcast(x, bf16), h[GATE + 16:]], axis=0)
        return _dot(h, wqkv_s[g, t, ks, :])

    def proj_store(n, t, y):
        i, g = n // G, n % G
        done = []
        if t == 0:
            q_s[n % 2] = (y * QSCALE).astype(bf16)
        elif t == 1:
            k_s[g, rows_of(i, R), :] = y.astype(bf16)
        else:
            for j in range(NQ):
                yt = y[j * 128:(j + 1) * 128].astype(bf16).T
                vt_s[g, i * NQ + j] = yt
                done.append(yt)
        return done

    def o_load(p):
        return jnp.concatenate([o_s[g, rows_of(p, PR), :] for g in range(G)], axis=1)

    def oproj_half(o, half):
        return _dot(o, wo_s[:, pl.ds(half * (D // 2), D // 2)])

    def shift_sel(bit, hi, lo):
        if hi is None and lo is None:
            return None
        ref = lo if hi is None else hi
        lane = lax.broadcasted_iota(i32, ref.shape, 1)
        zero = jnp.zeros_like(ref)
        return jnp.where(lane & (DH * bit) != 0, zero if hi is None else hi,
                         zero if lo is None else lo)

    def lane_rolls(x):
        x = pltpu.bitcast(x, u32)
        return [x] + [pltpu.roll(x, DH * s, 1) for s in range(1, HPG)]

    def attn_load(n, first_block):
        i, g = n // G, n % G
        back = 0 if first_block else WIN // 128
        qr = lane_rolls(q_s[n % 2])
        kr = lane_rolls(k_s[g, pl.ds(pl.multiple_of(i * R - back * 128, 128), R + back * 128), :])
        vt = {t: vt_s[g, i * NQ + t] for t in range(-back, NQ)}
        lo = -back * HPG
        kc = [{c + lo: x[c * 16:(c + 1) * 16] for c in range(x.shape[0] // 16)} for x in kr]
        u = [{c: shift_sel(1, kc[(s + 1) % HPG].get(c + 1), kc[s].get(c))
              for c in range(-NW, R // DH - 1)} for s in range(HPG)]
        ks = [{c: shift_sel(2, u[(2 - h) % HPG][c + 2], u[-h % HPG][c])
               for c in range(-NW, R // DH - 3)} for h in range(HPG)]
        return qr, ks, vt

    def qk(qr, ks, j, h, chunks, tok):
        w = []
        for a in range(HPG):
            x = qr[(a - h) % HPG][j * 64 + a * 16:j * 64 + (a + 1) * 16]
            lane = lax.broadcasted_iota(i32, x.shape, 1)
            w.append(jnp.where(lane // DH == a, x, jnp.zeros_like(x)))
        if tok is not None:
            w[0] = w[0] | jnp.concatenate([tok] * 2, axis=0)
        w = pltpu.bitcast(jnp.concatenate(w, axis=0), bf16)
        k = pltpu.bitcast(jnp.concatenate([ks[h][j * HPG - NW + c] for c in chunks], axis=0), bf16)
        s = lax.dot_general(k, w, (((1,), (1,)), ((), ())), preferred_element_type=f32)
        return {c: s[a * DH:(a + 1) * DH] for a, c in enumerate(chunks)}

    def softmax(ss, start, pace, zv):
        lane = lax.broadcasted_iota(i32, (DH, 128), 1)
        tri = lax.broadcasted_iota(i32, (DH, 128), 0) <= lane % DH
        wrap = 0 in ss[0]
        ms = []
        for s in ss:
            s[NW] = jnp.where(tri, s[NW], s.pop(0) if wrap else -jnp.inf)
            m = None
            for c in s:
                if c < start:
                    s[c] = jnp.where(lane // DH >= start - c, s[c], -jnp.inf)
                d = jnp.max(s[c].reshape(DH // 8, 8, 128), axis=0)
                m = d if m is None else jnp.maximum(m, d)
            ms.append(jnp.broadcast_to(jnp.max(m, axis=0, keepdims=True), (8, 128)))
        ls, es, mp = [None] * len(ss), [{} for _ in ss], list(ms)
        for a, c in enumerate(ss[0]):
            for h, s in enumerate(ss):
                if pace is not None and a % PACE == 0:
                    pr = pace.shape[0]
                    r0 = int((a + PACE * h / len(ss)) * pace.size // 128 * PFRAC)
                    r0 = r0 // len(s) // 8 * 8
                    src = pace[r0 % pr:r0 % pr + 8, r0 // pr * 128:(r0 // pr + 1) * 128]
                    mp[h] = pltpu.bitcast(
                        pltpu.bitcast(ms[h], u32) | (pltpu.bitcast(src, u32) & zv), f32)
                x = jnp.exp2(s[c].reshape(DH // 8, 8, 128) - mp[h])
                t = jnp.sum(x, axis=0)
                ls[h] = t if ls[h] is None else ls[h] + t
                es[h][c] = x.reshape(DH, 128)
        out = []
        for e, l in zip(es, ls):
            if wrap:
                x = e[NW]
                e[NW] = jnp.where(tri, x, 0.0)
                e[0] = x - e[NW]
            t = {c: shift_sel(1, e.get(c - 1), e.get(c)) for c in range(NW + 2)}
            p = {c: shift_sel(2, t.get(c - 2), t.get(c)) for c in range(max(start, 0), NW + HPG)}
            p = {c // HPG - WIN // 128: jnp.concatenate([p[c + a] for a in range(HPG)], axis=0)
                 for c in range(max(start, 0), NW + HPG, HPG)}
            out.append((p, jnp.sum(l, axis=0, keepdims=True)))
        return out

    def steps(n0, plans, first_block=False):
        oi = None if first_block else o_load(n0 - G)
        due = []
        for a, plan in enumerate(plans):
            oi = step(n0 + a, plan, first_block, oi, due, a + 1 < len(plans) and not first_block)

    def step(n, plan, first_block, oi, due, more):
        zv = zero_s[...]
        qr, ks, vt = attn_load(n, first_block)
        part, ss, sm = {}, {}, {}
        pace = None

        def settle():
            now = [x for wait, x in due if wait == 0]
            due[:] = [(wait - 1, x) for wait, x in due if wait]
            tok = zv if now else None
            for x in now:
                tok = tok & pltpu.bitcast(x[-32 // x.dtype.itemsize:, -128:], u32)
            return tok

        for op in plan.split():
            kind, j = op[0], int(op[1:])
            start = NW - j * HPG if first_block else 0
            if kind == "o":
                piece = n - G + j // 2
                if j > 1 and j % 2 == 0:
                    oi = o_load(piece)
                pace = oproj_half(oi, j % 2)
                if j % 2:
                    done = epilogue(jnp.concatenate([part["o"], pace], axis=1), piece)
                    due.extend((EPI_WAIT, x) for x in done)
                part["o"] = pace
            elif kind == "N":
                ln_store(ln_load((n + LEAD) % NP), (n + LEAD) % NP)
            elif kind in "QKV":
                t = "QKV".index(kind)
                pace = proj_half(n + 1, t, j, settle())
                if j:
                    due.extend((0, x) for x in proj_store(n + 1, t, part[t] + pace))
                part[t] = pace
            elif kind == "s":
                chunks = ([0] if start <= 0 else []) + [NW]
                chunks += range(max(start - HPG + 1, 1), NW)
                tok = None
                if pace is not None:
                    tok = pltpu.bitcast(pace[0:8, 0:128], u32) & zv
                ss[j] = [qk(qr, ks, j, h, chunks, tok) for h in range(HPG)]
                pace = None
            elif kind == "e":
                sm[j] = softmax(ss[j], start, pace, zv)
            else:
                if more and j == NQ - 1:
                    o_next = o_load(n + 1 - G)
                ot = [None] * HPG
                for t in sm[j][0][0]:
                    for h, (p, _) in enumerate(sm[j]):
                        y = _dot(vt[j + t][h * DH:(h + 1) * DH], p[t].astype(bf16))
                        ot[h] = y if ot[h] is None else ot[h] + y
                ot = jnp.concatenate([y * (1.0 / l) for y, (_, l) in zip(ot, sm[j])], axis=0)
                ot = ot.astype(bf16).T
                o_s[n % G, rows_of((n // G) * NQ + j, 128), :] = ot
                due.append((0, ot))
        return o_next if more else None


    x_in(0).wait()
    for c in wqkv_in(0):
        c.start()

    def ln_head(p, c):
        ln_store(ln_load(p), p)
        return c
    lax.fori_loop(0, LEAD, ln_head, 0, unroll=3)
    x_in(1).start()
    for g in range(1, 1 + HEAD_U):
        for c in wqkv_in(g):
            c.start()
    wqkv_wait(0)

    def layer(li, carry):
        first, last = li == 0, li == LAYERS - 1
        best_s[...] = jnp.full(best_s.shape, -jnp.inf, f32)
        bidx_s[...] = jnp.zeros_like(bidx_s)

        for t in (2, 1, 0):
            proj_store(0, t, proj_half(0, t, 0) + proj_half(0, t, 1))

        def head_body(a, c):
            n = a * HEAD_U
            for n0 in range(0, G, HEAD_U):
                @pl.when(first & (n == n0))
                def _():
                    for g in range(n0 + 1, min(n0 + 1 + HEAD_U, G)):
                        wqkv_wait(g)
                    for g in range(n0 + 1 + HEAD_U, min(n0 + 1 + 2 * HEAD_U, G)):
                        for c in wqkv_in(g):
                            c.start()
                    if n0 == 0:
                        x_in(1).wait()
                        x_in(2).start()
                    if n0 == HEAD_U:
                        x_in(2).wait()
                        wo_in.start()

            steps(n, [PLAN_HEAD] * HEAD_U, first_block=True)
            return c
        lax.fori_loop(0, G // HEAD_U, head_body, 0)

        @pl.when(first)
        def _():
            wo_in.wait()
            for c in ffn_in:
                c.start()

        def body(a, c):
            n = a * BODY_U
            for b in range(NB - 2):
                @pl.when(last & (n == G * (b + 2)))
                def _():
                    x_out(b).start()

            steps(n, [PLAN_BODY] * BODY_U)
            return c
        lax.fori_loop(G // BODY_U, NSTEP // BODY_U - 1, body, 0)

        @pl.when(first)
        def _():
            for c in ffn_in:
                c.wait()

        steps(NSTEP - BODY_U, [PLAN_BODY] * (BODY_U - 1) + [PLAN_LAST])

        @pl.when(last)
        def _():
            for b in range(NB - 2, NB):
                x_out(b).start()

        best = best_s[...]
        top = jnp.max(best, axis=0, keepdims=True)
        idx = jnp.clip(jnp.min(jnp.where(best == top, bidx_s[...], S)), 0, S - 1)
        slab = rows_of(idx // 16, 16)
        sel = lax.broadcasted_iota(i32, (16, D), 0) == idx % 16
        hs = h1_s[slab, :]
        gate = _dot(hs, wg_s[...])
        up = _dot(hs, wu_s[...])
        y = _dot((gate * jax.nn.sigmoid(gate) * up).astype(bf16), wd_s[:, 0:D])
        y = y * jax.nn.sigmoid(top[:, 0:1])

        @pl.when(last)
        def _():
            for b in range(NB):
                x_out(b).wait()

        xs = x_s[slab, :].astype(f32)
        xs = jnp.where(sel, xs + y, xs).astype(bf16)
        x_s[slab, :] = xs

        @pl.when(last)
        def _():
            c = pltpu.make_async_copy(x_s.at[slab], out_hbm.at[slab], sem_o.at[0])
            c.start()
            c.wait()

        h_s[slab, :] = _ln(xs.astype(f32)).astype(bf16)
        return carry

    lax.fori_loop(0, LAYERS, layer, 0)


@jax.jit
def pallas_interleave_layers__sliding_block__moe_arch_mod__prompt_kernel(
    A_x: jax.Array,
    A_wqkv: jax.Array,
    A_wo: jax.Array,
    B_x: jax.Array,
    B_w_r: jax.Array,
    B_w_gate: jax.Array,
    B_w_up: jax.Array,
    B_w_down: jax.Array,
):
    del B_x
    hbm = pl.BlockSpec(memory_space=pl.ANY)
    out = pl.pallas_call(
        _kernel,
        in_specs=[hbm, hbm, hbm, pl.BlockSpec(memory_space=pltpu.VMEM), hbm, hbm, hbm],
        out_specs=hbm,
        out_shape=jax.ShapeDtypeStruct((S, D), bf16),
        scratch_shapes=[
            pltpu.VMEM((S, D), bf16),
            pltpu.VMEM((S, D), bf16),
            pltpu.VMEM((S, D), bf16),
            pltpu.VMEM((2, R, 128), bf16),
            pltpu.VMEM((G, S, 128), bf16),
            pltpu.VMEM((G, S // 128, 128, 128), bf16),
            pltpu.VMEM((G, S, 128), bf16),
            pltpu.VMEM((G, 3, D, 128), bf16),
            pltpu.VMEM((D, D + 128), bf16),
            pltpu.VMEM((D, F), bf16),
            pltpu.VMEM((D, F), bf16),
            pltpu.VMEM((F, D + 128), bf16),
            pltpu.VMEM((8, 128), f32),
            pltpu.VMEM((8, 128), i32),
            pltpu.VMEM((8, 128), u32),
            pltpu.VMEM((8, D), f32),
            pltpu.SemaphoreType.DMA((3,)),
            pltpu.SemaphoreType.DMA((G + 4,)),
            pltpu.SemaphoreType.DMA((NB,)),
        ],
        compiler_params=pltpu.CompilerParams(vmem_limit_bytes=100 * 1024 * 1024),
    )(A_x.reshape(S, D), A_wqkv, A_wo, B_w_r,
      B_w_gate, B_w_up, B_w_down)
    return out.reshape(1, S, D)
```

```python
import math

import jax
import jax.numpy as jnp
from jax import lax
import jax.experimental.pallas as pl
import jax.experimental.pallas.tpu as pltpu

S, D, F = 2048, 1024, 3584
DH = 32
HPG = 4
G = D // 128
R = 512
NQ = R // 128
NB = S // R
PR = R // G
NP = S // PR
NSTEP = NB * G
LAYERS = 2
EPS = 1e-5
WIN = 256
NW = WIN // DH
HEAD_U, BODY_U = 2, 2
PACE, PFRAC = 4, 0.65
GATE = 416
EPI_WAIT = 3
PLAN_HEAD = "V0 s3 K0 e3 p3 s0 V1 e0 p0 N0 s2 Q0 e2 p2 s1 Q1 e1 p1 K1"
PLAN_BODY = "o0 N0 o1 s0 V0 e0 p0 Q0 s1 K0 e1 p1 s2 K1 e2 p2 s3 V1 e3 p3 Q1"
PLAN_LAST = ("s0 o0 e0 o1 p0 s1 o2 e1 o3 N0 o4 p1 s2 o5 e2 o6 o7 p2 o8 s3 o9 e3 o10 o11 o12 p3 "
             "o13 o14 o15 o16 o17")
LEAD = G + 1
QSCALE = DH ** -0.5 * math.log2(math.e)

bf16 = jnp.bfloat16
f32 = jnp.float32
u32 = jnp.uint32
i32 = jnp.int32


def _ln(x):
    m = jnp.mean(x, axis=-1, keepdims=True)
    xc = x - m
    v = jnp.mean(xc * xc, axis=-1, keepdims=True)
    return xc * lax.rsqrt(v + EPS)


def _dot(a, b):
    return jnp.dot(a, b, preferred_element_type=f32)


def _kernel(x_hbm, wqkv_hbm, wo_hbm, wr_ref, wg_hbm, wu_hbm, wd_hbm, out_hbm,
            x_s, h_s, h1_s, q_s, k_s, vt_s, o_s, wqkv_s, wo_s, wg_s, wu_s, wd_s,
            best_s, bidx_s, zero_s, wr_s, sem_x, sem_w, sem_o):

    def x_in(b):
        edges = (0, 3 * PR, 6 * PR, LEAD * PR, (LEAD + HEAD_U) * PR, S)
        rows = pl.ds(edges[b], edges[b + 1] - edges[b])
        return pltpu.make_async_copy(x_hbm.at[rows], x_s.at[rows], sem_x.at[b])

    def wqkv_in(g):
        return [pltpu.make_async_copy(
            wqkv_hbm.at[:, pl.ds(t * D + g * 128, 128)], wqkv_s.at[g, t], sem_w.at[g])
            for t in range(3)]

    def wqkv_wait(g):
        pltpu.make_async_copy(wqkv_s.at[g], wqkv_s.at[g], sem_w.at[g]).wait()

    wo_in = pltpu.make_async_copy(wo_hbm, wo_s.at[:, 0:D], sem_w.at[G])
    ffn_in = [pltpu.make_async_copy(a, b, sem_w.at[G + 1 + i]) for i, (a, b) in
              enumerate(((wg_hbm, wg_s), (wu_hbm, wu_s), (wd_hbm, wd_s.at[:, 0:D])))]

    def x_out(b):
        rows = pl.ds(b * R, R)
        return pltpu.make_async_copy(x_s.at[rows], out_hbm.at[rows], sem_o.at[b])

    for b in range(3):
        x_in(b).start()
    wr_s[...] = jnp.broadcast_to(wr_ref[...].astype(f32).reshape(1, D), (8, D))
    zero_s[...] = jnp.zeros_like(zero_s)

    def rows_of(p, n):
        return pl.ds(p * n if isinstance(p, int) else pl.multiple_of(p * n, n), n)

    def ln_load(p):
        return x_s[rows_of(p, PR), :].astype(f32)

    def ln_store(x, p):
        h_s[rows_of(p, PR), :] = _ln(x).astype(bf16)

    def epilogue(y, p):
        x1 = ln_load(p) + y
        xc = x1 - jnp.mean(x1, axis=-1, keepdims=True)
        rstd = lax.rsqrt(jnp.mean(xc * xc, axis=-1, keepdims=True) + EPS)
        r = jnp.sum(xc * wr_s[0:1, :], axis=-1, keepdims=True) * rstd
        h1 = xc * rstd
        xb = (x1 + h1).astype(bf16)
        x_s[rows_of(p, PR), :] = xb
        h1_s[rows_of(p, PR), :] = h1.astype(bf16)
        r = jnp.broadcast_to(r, (PR, 128))
        best, bidx = best_s[...], bidx_s[...]
        row = lax.broadcasted_iota(i32, (8, 128), 0) + p * PR
        for t in range(PR // 8):
            rt = r[t * 8:(t + 1) * 8]
            up = rt > best
            best = jnp.where(up, rt, best)
            bidx = jnp.where(up, row + t * 8, bidx)
        best_s[...] = best
        bidx_s[...] = bidx
        return [bidx] + [xb[:r] for r in range(16, PR + 1, 16)]

    def proj_half(n, t, half, tok=None):
        i, g = n // G, n % G
        ks = pl.ds(half * (D // 2), D // 2)
        h = h_s[rows_of(i, R), ks]
        if tok is not None:
            x = pltpu.bitcast(h[GATE:GATE + 16], u32) | jnp.concatenate([tok] * (D // 256), axis=1)
            h = jnp.concatenate([h[:GATE], pltpu.bitcast(x, bf16), h[GATE + 16:]], axis=0)
        return _dot(h, wqkv_s[g, t, ks, :])

    def proj_store(n, t, y):
        i, g = n // G, n % G
        done = []
        if t == 0:
            q_s[n % 2] = (y * QSCALE).astype(bf16)
        elif t == 1:
            k_s[g, rows_of(i, R), :] = y.astype(bf16)
        else:
            for j in range(NQ):
                yt = y[j * 128:(j + 1) * 128].astype(bf16).T
                vt_s[g, i * NQ + j] = yt
                done.append(yt)
        return done

    def o_load(p):
        return jnp.concatenate([o_s[g, rows_of(p, PR), :] for g in range(G)], axis=1)

    def oproj_half(o, half):
        return _dot(o, wo_s[:, pl.ds(half * (D // 2), D // 2)])

    def shift_sel(bit, hi, lo):
        if hi is None and lo is None:
            return None
        ref = lo if hi is None else hi
        lane = lax.broadcasted_iota(i32, ref.shape, 1)
        zero = jnp.zeros_like(ref)
        return jnp.where(lane & (DH * bit) != 0, zero if hi is None else hi,
                         zero if lo is None else lo)

    def lane_rolls(x):
        x = pltpu.bitcast(x, u32)
        return [x] + [pltpu.roll(x, DH * s, 1) for s in range(1, HPG)]

    def attn_load(n, first_block):
        i, g = n // G, n % G
        back = 0 if first_block else WIN // 128
        qr = lane_rolls(q_s[n % 2])
        kr = lane_rolls(k_s[g, pl.ds(pl.multiple_of(i * R - back * 128, 128), R + back * 128), :])
        vt = {t: vt_s[g, i * NQ + t] for t in range(-back, NQ)}
        lo = -back * HPG
        kc = [{c + lo: x[c * 16:(c + 1) * 16] for c in range(x.shape[0] // 16)} for x in kr]
        u = [{c: shift_sel(1, kc[(s + 1) % HPG].get(c + 1), kc[s].get(c))
              for c in range(-NW, R // DH - 1)} for s in range(HPG)]
        ks = [{c: shift_sel(2, u[(2 - h) % HPG][c + 2], u[-h % HPG][c])
               for c in range(-NW, R // DH - 3)} for h in range(HPG)]
        return qr, ks, vt

    def qk(qr, ks, j, h, chunks, tok):
        w = []
        for a in range(HPG):
            x = qr[(a - h) % HPG][j * 64 + a * 16:j * 64 + (a + 1) * 16]
            lane = lax.broadcasted_iota(i32, x.shape, 1)
            w.append(jnp.where(lane // DH == a, x, jnp.zeros_like(x)))
        if tok is not None:
            w[0] = w[0] | jnp.concatenate([tok] * 2, axis=0)
        w = pltpu.bitcast(jnp.concatenate(w, axis=0), bf16)
        k = pltpu.bitcast(jnp.concatenate([ks[h][j * HPG - NW + c] for c in chunks], axis=0), bf16)
        s = lax.dot_general(k, w, (((1,), (1,)), ((), ())), preferred_element_type=f32)
        return {c: s[a * DH:(a + 1) * DH] for a, c in enumerate(chunks)}

    def softmax(ss, start, pace, zv):
        lane = lax.broadcasted_iota(i32, (DH, 128), 1)
        tri = lax.broadcasted_iota(i32, (DH, 128), 0) <= lane % DH
        wrap = 0 in ss[0]
        ms = []
        for s in ss:
            s[NW] = jnp.where(tri, s[NW], s.pop(0) if wrap else -jnp.inf)
            m = None
            for c in s:
                if c < start:
                    s[c] = jnp.where(lane // DH >= start - c, s[c], -jnp.inf)
                d = jnp.max(s[c].reshape(DH // 8, 8, 128), axis=0)
                m = d if m is None else jnp.maximum(m, d)
            ms.append(jnp.broadcast_to(jnp.max(m, axis=0, keepdims=True), (8, 128)))
        ls, es, mp = [None] * len(ss), [{} for _ in ss], list(ms)
        for a, c in enumerate(ss[0]):
            for h, s in enumerate(ss):
                if pace is not None and a % PACE == 0:
                    pr = pace.shape[0]
                    r0 = int((a + PACE * h / len(ss)) * pace.size // 128 * PFRAC)
                    r0 = r0 // len(s) // 8 * 8
                    src = pace[r0 % pr:r0 % pr + 8, r0 // pr * 128:(r0 // pr + 1) * 128]
                    mp[h] = pltpu.bitcast(
                        pltpu.bitcast(ms[h], u32) | (pltpu.bitcast(src, u32) & zv), f32)
                x = jnp.exp2(s[c].reshape(DH // 8, 8, 128) - mp[h])
                t = jnp.sum(x, axis=0)
                ls[h] = t if ls[h] is None else ls[h] + t
                es[h][c] = x.reshape(DH, 128)
        out = []
        for e, l in zip(es, ls):
            if wrap:
                x = e[NW]
                e[NW] = jnp.where(tri, x, 0.0)
                e[0] = x - e[NW]
            t = {c: shift_sel(1, e.get(c - 1), e.get(c)) for c in range(NW + 2)}
            p = {c: shift_sel(2, t.get(c - 2), t.get(c)) for c in range(max(start, 0), NW + HPG)}
            p = {c // HPG - WIN // 128: jnp.concatenate([p[c + a] for a in range(HPG)], axis=0)
                 for c in range(max(start, 0), NW + HPG, HPG)}
            out.append((p, jnp.sum(l, axis=0, keepdims=True)))
        return out

    def steps(n0, plans, first_block=False):
        oi = None if first_block else o_load(n0 - G)
        due = []
        for a, plan in enumerate(plans):
            oi = step(n0 + a, plan, first_block, oi, due, a + 1 < len(plans) and not first_block)

    def step(n, plan, first_block, oi, due, more):
        zv = zero_s[...]
        qr, ks, vt = attn_load(n, first_block)
        part, ss, sm = {}, {}, {}
        pace = None

        def settle():
            now = [x for wait, x in due if wait == 0]
            due[:] = [(wait - 1, x) for wait, x in due if wait]
            tok = zv if now else None
            for x in now:
                tok = tok & pltpu.bitcast(x[-32 // x.dtype.itemsize:, -128:], u32)
            return tok

        for op in plan.split():
            kind, j = op[0], int(op[1:])
            start = NW - j * HPG if first_block else 0
            if kind == "o":
                piece = n - G + j // 2
                if j > 1 and j % 2 == 0:
                    oi = o_load(piece)
                pace = oproj_half(oi, j % 2)
                if j % 2:
                    done = epilogue(jnp.concatenate([part["o"], pace], axis=1), piece)
                    due.extend((EPI_WAIT, x) for x in done)
                part["o"] = pace
            elif kind == "N":
                ln_store(ln_load((n + LEAD) % NP), (n + LEAD) % NP)
            elif kind in "QKV":
                t = "QKV".index(kind)
                pace = proj_half(n + 1, t, j, settle())
                if j:
                    due.extend((0, x) for x in proj_store(n + 1, t, part[t] + pace))
                part[t] = pace
            elif kind == "s":
                chunks = ([0] if start <= 0 else []) + [NW]
                chunks += range(max(start - HPG + 1, 1), NW)
                tok = None
                if pace is not None:
                    tok = pltpu.bitcast(pace[0:8, 0:128], u32) & zv
                ss[j] = [qk(qr, ks, j, h, chunks, tok) for h in range(HPG)]
                pace = None
            elif kind == "e":
                sm[j] = softmax(ss[j], start, pace, zv)
            else:
                if more and j == NQ - 1:
                    o_next = o_load(n + 1 - G)
                ot = [None] * HPG
                for t in sm[j][0][0]:
                    for h, (p, _) in enumerate(sm[j]):
                        y = _dot(vt[j + t][h * DH:(h + 1) * DH], p[t].astype(bf16))
                        ot[h] = y if ot[h] is None else ot[h] + y
                ot = jnp.concatenate([y * (1.0 / l) for y, (_, l) in zip(ot, sm[j])], axis=0)
                ot = ot.astype(bf16).T
                o_s[n % G, rows_of((n // G) * NQ + j, 128), :] = ot
                due.append((0, ot))
        return o_next if more else None

    for b in range(3):
        x_in(b).wait()
        if b == 0:
            for c in wqkv_in(0):
                c.start()
        if b == 2:
            x_in(3).start()
            for g in range(1, 1 + HEAD_U):
                for c in wqkv_in(g):
                    c.start()
        for p in range(3 * b, 3 * b + 3):
            ln_store(ln_load(p), p)
    wqkv_wait(0)

    def layer(li, carry):
        first, last = li == 0, li == LAYERS - 1
        best_s[...] = jnp.full(best_s.shape, -jnp.inf, f32)
        bidx_s[...] = jnp.zeros_like(bidx_s)

        for t in (2, 1, 0):
            proj_store(0, t, proj_half(0, t, 0) + proj_half(0, t, 1))

        def head_body(a, c):
            n = a * HEAD_U
            for n0 in range(0, G, HEAD_U):
                @pl.when(first & (n == n0))
                def _():
                    for g in range(n0 + 1, min(n0 + 1 + HEAD_U, G)):
                        wqkv_wait(g)
                    for g in range(n0 + 1 + HEAD_U, min(n0 + 1 + 2 * HEAD_U, G)):
                        for c in wqkv_in(g):
                            c.start()
                    if n0 == 0:
                        x_in(3).wait()
                        x_in(4).start()
                    if n0 == HEAD_U:
                        x_in(4).wait()
                        wo_in.start()

            steps(n, [PLAN_HEAD] * HEAD_U, first_block=True)
            return c
        lax.fori_loop(0, G // HEAD_U, head_body, 0)

        @pl.when(first)
        def _():
            wo_in.wait()
            for c in ffn_in:
                c.start()

        def body(a, c):
            n = a * BODY_U
            for b in range(NB - 2):
                @pl.when(last & (n == G * (b + 2)))
                def _():
                    x_out(b).start()

            steps(n, [PLAN_BODY] * BODY_U)
            return c
        lax.fori_loop(G // BODY_U, NSTEP // BODY_U - 1, body, 0)

        @pl.when(first)
        def _():
            for c in ffn_in:
                c.wait()

        steps(NSTEP - BODY_U, [PLAN_BODY] * (BODY_U - 1) + [PLAN_LAST])

        @pl.when(last)
        def _():
            for b in range(NB - 2, NB):
                x_out(b).start()

        best = best_s[...]
        top = jnp.max(best, axis=0, keepdims=True)
        idx = jnp.clip(jnp.min(jnp.where(best == top, bidx_s[...], S)), 0, S - 1)
        slab = rows_of(idx // 16, 16)
        sel = lax.broadcasted_iota(i32, (16, D), 0) == idx % 16
        hs = h1_s[slab, :]
        gate = _dot(hs, wg_s[...])
        up = _dot(hs, wu_s[...])
        y = _dot((gate * jax.nn.sigmoid(gate) * up).astype(bf16), wd_s[:, 0:D])
        y = y * jax.nn.sigmoid(top[:, 0:1])

        @pl.when(last)
        def _():
            for b in range(NB):
                x_out(b).wait()

        xs = x_s[slab, :].astype(f32)
        xs = jnp.where(sel, xs + y, xs).astype(bf16)
        x_s[slab, :] = xs

        @pl.when(last)
        def _():
            c = pltpu.make_async_copy(x_s.at[slab], out_hbm.at[slab], sem_o.at[0])
            c.start()
            c.wait()

        h_s[slab, :] = _ln(xs.astype(f32)).astype(bf16)
        return carry

    lax.fori_loop(0, LAYERS, layer, 0)


@jax.jit
def pallas_interleave_layers__sliding_block__moe_arch_mod__prompt_kernel(
    A_x: jax.Array,
    A_wqkv: jax.Array,
    A_wo: jax.Array,
    B_x: jax.Array,
    B_w_r: jax.Array,
    B_w_gate: jax.Array,
    B_w_up: jax.Array,
    B_w_down: jax.Array,
):
    del B_x
    hbm = pl.BlockSpec(memory_space=pl.ANY)
    out = pl.pallas_call(
        _kernel,
        in_specs=[hbm, hbm, hbm, pl.BlockSpec(memory_space=pltpu.VMEM), hbm, hbm, hbm],
        out_specs=hbm,
        out_shape=jax.ShapeDtypeStruct((S, D), bf16),
        scratch_shapes=[
            pltpu.VMEM((S, D), bf16),
            pltpu.VMEM((S, D), bf16),
            pltpu.VMEM((S, D), bf16),
            pltpu.VMEM((2, R, 128), bf16),
            pltpu.VMEM((G, S, 128), bf16),
            pltpu.VMEM((G, S // 128, 128, 128), bf16),
            pltpu.VMEM((G, S, 128), bf16),
            pltpu.VMEM((G, 3, D, 128), bf16),
            pltpu.VMEM((D, D + 128), bf16),
            pltpu.VMEM((D, F), bf16),
            pltpu.VMEM((D, F), bf16),
            pltpu.VMEM((F, D + 128), bf16),
            pltpu.VMEM((8, 128), f32),
            pltpu.VMEM((8, 128), i32),
            pltpu.VMEM((8, 128), u32),
            pltpu.VMEM((8, D), f32),
            pltpu.SemaphoreType.DMA((5,)),
            pltpu.SemaphoreType.DMA((G + 4,)),
            pltpu.SemaphoreType.DMA((NB,)),
        ],
        compiler_params=pltpu.CompilerParams(vmem_limit_bytes=100 * 1024 * 1024),
    )(A_x.reshape(S, D), A_wqkv, A_wo, B_w_r,
      B_w_gate, B_w_up, B_w_down)
    return out.reshape(1, S, D)
```
